```python
import jax
import jax.numpy as jnp

def _softmax(x, axis=-1):
    return jax.nn.softmax(x, axis=axis)
def _gelu(x):
    return jax.nn.gelu(x, approximate=True)
def _silu(x):
    return jax.nn.silu(x)
def _sigmoid(x):
    return jax.nn.sigmoid(x)
def _layernorm(x, axis=-1, eps=1e-5):
    m = jnp.mean(x, axis=axis, keepdims=True)
    v = jnp.var(x, axis=axis, keepdims=True)
    return (x - m) / jnp.sqrt(v + eps)
def _scatter_add(tgt, idx, src, axis=0):
    return tgt.at[idx].add(src)
def _segment_sum(src, seg, n):
    return jax.ops.segment_sum(src, seg, n)
class _Rng:
    def __init__(self, key):
        self._k = key
    def _next(self):
        self._k, sub = jax.random.split(self._k)
        return sub
    def normal(self, shape):
        return jax.random.normal(self._next(), shape, dtype=jnp.bfloat16)
    def randint(self, lo, hi, shape):
        return jax.random.randint(self._next(), shape, lo, hi, dtype=jnp.int32)
    def uniform(self, shape, lo=0.0, hi=1.0):
        return jax.random.uniform(self._next(), shape, jnp.bfloat16, lo, hi)
    def permutation(self, n):
        return jax.random.permutation(self._next(), n)


kernel_name = 'recurrent_scan__sliding_local_dilated__glu_gated_swiglu__prompt'

def setup_inputs():
    _rng = _Rng(jax.random.key(int.from_bytes(__import__("os").urandom(4), "little")))
    _w = (lambda a: (lambda t: t.astype(jnp.bfloat16) if jnp.issubdtype(t.dtype, jnp.floating) else t)(jnp.asarray(a)))
    def _A_setup():
        B, S, D = 1, 2048, 1024
        return {
            "x": _w((lambda *s: _rng.normal(s) * 0.05)(B, S, D)),
            "wqkv": _w((lambda *s: _rng.normal(s) * 0.05)(D, 3 * D)),
            "wo": _w((lambda *s: _rng.normal(s) * 0.05)(D, D)),
        }
    _A_in = _A_setup()

    def _B_setup():
        B, S, D, F = 1, 2048, 1024, 3584
        return {
            "x": _w((lambda *s: _rng.normal(s) * 0.05)(B, S, D)),
            "w1": _w((lambda *s: _rng.normal(s) * 0.05)(D, F) * (2.0 / D) ** 0.5),
            "w3": _w((lambda *s: _rng.normal(s) * 0.05)(D, F) * (2.0 / D) ** 0.5),
            "w2": _w((lambda *s: _rng.normal(s) * 0.05)(F, D) * (2.0 / F) ** 0.5),
        }
    _B_in = _B_setup()

    return {
        "A_x": _A_in["x"],
        "A_wqkv": _A_in["wqkv"],
        "A_wo": _A_in["wo"],
        "B_x": _B_in["x"],
        "B_w1": _B_in["w1"],
        "B_w3": _B_in["w3"],
        "B_w2": _B_in["w2"],
    }

def reference(A_x, A_wqkv, A_wo, B_x, B_w1, B_w3, B_w2):
    def _A_ref(x, wqkv, wo):
        B, S, D = x.shape
        H = 32; Dh = D // H
        W, dil = 8, 2
        qkv = (lambda x, *d: x.transpose(*d))((x @ wqkv).reshape(B, S, 3, H, Dh), 2, 0, 3, 1, 4)
        q, k, v = qkv[0], qkv[1], qkv[2]
        scale = Dh ** -0.5
        pos = jnp.arange(S)
        off = jnp.arange(W) * dil
        idx = pos[:, None] - off[None, :]
        mask = idx >= 0
        idx_c = jnp.where(mask, idx, 0).reshape(-1)
        kg = k[:, :, idx_c, :].reshape(B, H, S, W, Dh)
        vg = v[:, :, idx_c, :].reshape(B, H, S, W, Dh)
        logits = jnp.einsum("bhsd,bhswd->bhsw", q, kg) * scale
        logits = jnp.where(mask[None, None, :, :], logits, -1e9)
        attn = _softmax(logits, axis=-1)
        o = jnp.einsum("bhsw,bhswd->bhsd", attn, vg)
        return (lambda x, *d: x.transpose(*d))(o, 0, 2, 1, 3).reshape(B, S, D) @ wo

    def _B_ref(x, w1, w3, w2):
        gate = jnp.einsum("bsd,df->bsf", x, w1)
        up = jnp.einsum("bsd,df->bsf", x, w3)
        h = _silu(gate) * up
        out = jnp.einsum("bsf,fd->bsd", h, w2)
        return out

    x = A_x
    xn = _layernorm(x, axis=-1)
    s = _A_ref(xn, A_wqkv, A_wo)
    g = _silu(_B_ref(xn, B_w1, B_w3, B_w2))
    return x + s * g
```

```python
import jax
import jax.numpy as jnp
import numpy as np
from jax.experimental import pallas as pl
from jax.experimental.pallas import tpu as pltpu
S,D,F=2048,1024,3584
f32=jnp.float32; bf16=jnp.bfloat16; i32=jnp.int32

def lane_field_masks(shape):
    lane=jax.lax.broadcasted_iota(i32,shape,len(shape)-1)
    fld=(lane>>1)&7
    return [((fld>>b)&1)==1 for b in range(3)]

def permute_fwd(cols):
    masks=lane_field_masks(cols[0].shape)
    R=[cols[c] if c==0 else pltpu.roll(cols[c],2*c,1) for c in range(8)]
    X=[R[(-c)%8] for c in range(8)]
    for b in range(3):
        sh=1<<b
        X=[jnp.where(masks[b],X[(j-sh)%8],X[j]) for j in range(8)]
    return [X[j] if j==0 else pltpu.roll(X[j],128-2*j,1) for j in range(8)]
permute_inv=permute_fwd

def mk(TM=512, mode='full', NIT=8, FC0=512, unit=16):
    FC=(F-FC0)//NIT
    assert FC0+NIT*FC==F and FC%128==0
    RPI=TM//NIT
    HALO=16
    scale=32**-0.5
    def kern(x_ref,wqkv_ref,wo_ref,w1_ref,w3_ref,w2_ref,o_ref,xn_s,q_s,k_s,v_s,ob_s,acc_s):
        i=pl.program_id(0)
        @pl.when(i==0)
        def _():
            k_s[:,0:HALO,:]=jnp.zeros((8,HALO,128),f32)
            v_s[:,0:HALO,:]=jnp.zeros((8,HALO,128),f32)
        @pl.when(i>0)
        def _():
            k_s[:,0:HALO,:]=k_s[:,TM:TM+HALO,:]
            v_s[:,0:HALO,:]=v_s[:,TM:TM+HALO,:]
        x=x_ref[...].astype(f32)
        m=jnp.mean(x,axis=-1,keepdims=True)
        xc=x-m
        var=jnp.mean(xc*xc,axis=-1,keepdims=True)
        xn_s[...]=(xc*jax.lax.rsqrt(var+1e-5)).astype(bf16)

        def ffn(sl,first):
            xn=xn_s[...]
            g=jnp.dot(xn,w1_ref[:,sl],preferred_element_type=f32)
            u=jnp.dot(xn,w3_ref[:,sl],preferred_element_type=f32)
            h=(g*jax.nn.sigmoid(g)*u).astype(bf16)
            d=jnp.dot(h,w2_ref[sl,:],preferred_element_type=f32)
            if first: acc_s[...]=d
            else: acc_s[...]+=d
        ffn(slice(0,FC0),True)
        for part,(dst,off) in enumerate(((q_s,0),(k_s,HALO),(v_s,HALO))):
            r=jnp.dot(xn_s[...],wqkv_ref[:,part*D:(part+1)*D],preferred_element_type=f32).astype(bf16)
            ri=pltpu.bitcast(r,i32)
            cols=permute_fwd([ri[:,c*128:(c+1)*128] for c in range(8)])
            for j in range(8):
                val=pltpu.bitcast(cols[j],bf16).astype(f32)
                if part==0: val=val*(scale*np.log2(np.e))
                dst[j,off:off+TM,:]=val

        def attn(b):
            R=unit
            row=jax.lax.broadcasted_iota(i32,(R,128),0)+(i*TM+b)
            lane=jax.lax.broadcasted_iota(i32,(R,128),1)
            b0=(lane&1)==1; b4=(lane&16)!=0
            q=[q_s[j,pl.ds(b,R),:] for j in range(8)]
            Z=[]
            for w in range(8):
                st=pl.ds(b+HALO-2*w,R)
                z=q[0]*k_s[0,st,:]
                for j in range(1,8): z=z+q[j]*k_s[j,st,:]
                z=z+jnp.where(b0,pltpu.roll(z,1,1),pltpu.roll(z,127,1))
                z=z+jnp.where(b4,pltpu.roll(z,16,1),pltpu.roll(z,112,1))
                if w>0: z=jnp.where(row>=2*w,z,-1e9)
                Z.append(z)
            mx=Z[0]
            for w in range(1,8): mx=jnp.maximum(mx,Z[w])
            E=[jnp.exp2(z-mx) for z in Z]
            den=E[0]
            for w in range(1,8): den=den+E[w]
            rden=1.0/den
            A=[e*rden for e in E]
            outs=[]
            for j in range(8):
                o=A[0]*v_s[j,pl.ds(b+HALO,R),:]
                for w in range(1,8): o=o+A[w]*v_s[j,pl.ds(b+HALO-2*w,R),:]
                outs.append(pltpu.bitcast(o.astype(bf16),i32))
            nat=permute_inv(outs)
            for c in range(8):
                ob_s[pl.ds(b,R),c*128:(c+1)*128]=pltpu.bitcast(nat[c],bf16)

        def body(f,c):
            st=FC0+f*FC
            ffn(pl.ds(pl.multiple_of(st,128),FC),False)
            if mode!='noattn':
                for uu in range(RPI//unit):
                    attn(pl.multiple_of(f*RPI+uu*unit,unit))
            return c
        jax.lax.fori_loop(0,NIT,body,0)
        s=jnp.dot(ob_s[...],wo_ref[...],preferred_element_type=f32)
        ff=acc_s[...]
        g=ff*jax.nn.sigmoid(ff)
        o_ref[...]=(x_ref[...].astype(f32)+s*g).astype(o_ref.dtype)
    c1=lambda shp:pl.BlockSpec(shp,lambda i:(0,0),pipeline_mode=pl.Buffered(1))
    @jax.jit
    def fn(x,wqkv,wo,bx,w1,w3,w2):
        out=pl.pallas_call(kern,grid=(S//TM,),
            in_specs=[pl.BlockSpec((TM,D),lambda i:(i,0)),c1((D,3*D)),c1((D,D)),c1((D,F)),c1((D,F)),c1((F,D))],
            out_specs=pl.BlockSpec((TM,D),lambda i:(i,0)),
            out_shape=jax.ShapeDtypeStruct((S,D),bf16),
            scratch_shapes=[pltpu.VMEM((TM,D),bf16),pltpu.VMEM((8,TM,128),f32),pltpu.VMEM((8,TM+HALO,128),f32),
                            pltpu.VMEM((8,TM+HALO,128),f32),pltpu.VMEM((TM,D),bf16),pltpu.VMEM((TM,D),f32)],
            compiler_params=pltpu.CompilerParams(dimension_semantics=("arbitrary",),vmem_limit_bytes=110*2**20))(x[0],wqkv,wo,w1,w3,w2)
        return out[None]
    return fn

_fn = mk()


@jax.jit
def pallas_recurrent_scan__sliding_local_dilated__glu_gated_swiglu__prompt_kernel(
    A_x, A_wqkv, A_wo, B_x, B_w1, B_w3, B_w2
):
    return _fn(A_x, A_wqkv, A_wo, B_x, B_w1, B_w3, B_w2)
```

```python
import contextlib
import jax
import jax.numpy as jnp
import numpy as np
from jax.experimental import pallas as pl
from jax.experimental.pallas import tpu as pltpu
S,D,F=2048,1024,3584
f32=jnp.float32; bf16=jnp.bfloat16; i32=jnp.int32
HALO=16

def lane_field_masks(shape):
    lane=jax.lax.broadcasted_iota(i32,shape,len(shape)-1)
    fld=(lane>>1)&7
    return [((fld>>b)&1)==1 for b in range(3)]

def permute(cols,masks):
    R=[cols[c] if c==0 else pltpu.roll(cols[c],2*c,1) for c in range(8)]
    X=[R[(-c)%8] for c in range(8)]
    for b in range(3):
        sh=1<<b
        X=[jnp.where(masks[b],X[(j-sh)%8],X[j]) for j in range(8)]
    return [X[j] if j==0 else pltpu.roll(X[j],128-2*j,1) for j in range(8)]

def silu_t(g):
    hg=0.5*g
    return hg+hg*jnp.tanh(hg)
def silu_e(g):
    return g*jax.nn.sigmoid(g)
def silu_a(g):
    return g*pl.reciprocal(1.0+jnp.exp(-g),approx=True)
def layernorm(x):
    x=x.astype(f32)
    m=jnp.mean(x,axis=-1,keepdims=True)
    xc=x-m
    var=jnp.mean(xc*xc,axis=-1,keepdims=True)
    return (xc*jax.lax.rsqrt(var+1e-5)).astype(bf16)

def mk(TM=512, FC0=512, NTRIP=4, SUB=2, unit=16, OB=2, mode='full', prof=False, lnrows=None, XP=2, stage=0, att_first=False, AHEAD=2, silu='tanh', inter=False, skipln=False):
    FT=(F-FC0)//NTRIP; FC=FT//SUB
    assert FC0+NTRIP*SUB*FC==F and FC%128==0
    RPT=TM//NTRIP
    NT=S//TM
    ORB=TM//OB
    XR=TM//XP
    silu_f={'tanh':silu_t,'exp':silu_e,'approx':silu_a}[silu]
    c_scale=float(32**-0.5*np.log2(np.e))
    sc=lambda n: jax.named_scope(n) if (prof is True or (prof and (n in prof or n.startswith('pro')))) else contextlib.nullcontext()
    def kern(x_hbm,wqkv_hbm,wo_hbm,w1_hbm,w3_hbm,w2_hbm,o_hbm,
             xb,wqkv_s,wo_s,w1_s,w3_s,w2_s,ob_out,xn_s,raw_s,kf_s,vf_s,ob_s,acc_s,xsem,osem,wsem,fsem):
        def xcopy(t,p):
            return pltpu.make_async_copy(x_hbm.at[pl.ds(pl.multiple_of(t*TM+p*XR,XR),XR),:],xb.at[t%2,pl.ds(p*XR,XR),:],xsem.at[t%2,p])
        def ocopy(t,r):
            return pltpu.make_async_copy(ob_out.at[t%2,pl.ds(r*ORB,ORB),:],o_hbm.at[pl.ds(pl.multiple_of(t*TM+r*ORB,ORB),ORB),:],osem.at[t%2,r])
        def fsl(f):
            if isinstance(f,int):
                return pl.ds(0,FC0) if f==0 else pl.ds(FC0+(f-1)*FT,FT)
            return pl.ds(pl.multiple_of(FC0+(f-1)*FT,128),FT)
        def w13copy(f):
            sl=fsl(f)
            return [pltpu.make_async_copy(w1_hbm.at[:,sl],w1_s.at[:,sl],fsem.at[0,f]),
                    pltpu.make_async_copy(w3_hbm.at[:,sl],w3_s.at[:,sl],fsem.at[1,f])]
        def w2copy(f):
            sl=fsl(f)
            return pltpu.make_async_copy(w2_hbm.at[sl,:],w2_s.at[sl,:],fsem.at[2,f])
        def qkvcopy(p):
            return pltpu.make_async_copy(wqkv_hbm.at[:,pl.ds(p*D,D)],wqkv_s.at[:,pl.ds(p*D,D)],wsem.at[p])
        def wocopy():
            return pltpu.make_async_copy(wo_hbm,wo_s,wsem.at[3])

        with sc('pro_issue'):
            for p in range(XP): xcopy(0,p).start()
            for c in w13copy(0): c.start()
            if stage==1: w2copy(0).start()
            raw_s[:,0:HALO,:]=jnp.zeros((2,HALO,D),bf16)
        for p in range(XP):
            with sc('pro_xwait'):
                xcopy(0,p).wait()
            with sc('pro_ln'):
                xn_s[0,p*XR:(p+1)*XR,:]=layernorm(xb[0,p*XR:(p+1)*XR,:])
        with sc('pro_wwait'):
            for c in w13copy(0): c.wait()
            if stage==0: w2copy(0).start()
            qkvcopy(0).start()
            if stage==2:
                w2copy(0).start()

        def tile(t,carry):
            slot=t%2
            first=t==0
            xn_t=xn_s.at[slot]
            def ffn(sl,init):
                g=jnp.dot(xn_t[...],w1_s[:,sl],preferred_element_type=f32)
                u=jnp.dot(xn_t[...],w3_s[:,sl],preferred_element_type=f32)
                h=(silu_f(g)*u).astype(bf16)
                d=jnp.dot(h,w2_s[sl,:],preferred_element_type=f32)
                if init: acc_s[...]=d
                else: acc_s[...]+=d
            with sc('w0wait'):
                @pl.when(first)
                def _():
                    w2copy(0).wait()
                    qkvcopy(1).start(); qkvcopy(2).start()
            with sc('ffn0'):
                ffn(slice(0,FC0),True)
            with sc('qkvwait'):
                @pl.when(first)
                def _():
                    for p in range(3): qkvcopy(p).wait()
                    for p in range(XP): xcopy(1,p).start()
                    for f in range(1,AHEAD+1):
                        for c in w13copy(f): c.start()
                        w2copy(f).start()
            with sc('qkv'):
                for part in range(3):
                    r=jnp.dot(xn_t[...],wqkv_s[:,part*D:(part+1)*D],preferred_element_type=f32).astype(bf16)
                    if part==0: ob_s[...]=r
                    else: raw_s[part-1,HALO:HALO+TM,:]=r

            def perm_kv(b):
                n=(RPT+HALO)
                masks=lane_field_masks((n//2,128))
                for part,dst in ((0,kf_s),(1,vf_s)):
                    ri=pltpu.bitcast(raw_s[part,pl.ds(b,n),:],i32)
                    cols=permute([ri[:,c*128:(c+1)*128] for c in range(8)],masks)
                    for j in range(8):
                        dst[j,:,:]=pltpu.bitcast(cols[j],bf16).astype(f32)

            def attn(b,lb):
                R=unit
                row=jax.lax.broadcasted_iota(i32,(R,128),0)+(t*TM+b)
                lane=jax.lax.broadcasted_iota(i32,(R,128),1)
                b0=(lane&1)==1; b4=(lane&16)!=0
                masks=lane_field_masks((R//2,128))
                qi=pltpu.bitcast(ob_s[pl.ds(b,R),:],i32)
                qc=permute([qi[:,c*128:(c+1)*128] for c in range(8)],masks)
                q=[pltpu.bitcast(c,bf16).astype(f32)*c_scale for c in qc]
                Z=[]
                for w in range(8):
                    st=pl.ds(lb+HALO-2*w,R)
                    z=q[0]*kf_s[0,st,:]
                    for j in range(1,8): z=z+q[j]*kf_s[j,st,:]
                    z=z+jnp.where(b0,pltpu.roll(z,1,1),pltpu.roll(z,127,1))
                    z=z+jnp.where(b4,pltpu.roll(z,16,1),pltpu.roll(z,112,1))
                    if w>0: z=jnp.where(row>=2*w,z,-1e9)
                    Z.append(z)
                mx=Z[0]
                for w in range(1,8): mx=jnp.maximum(mx,Z[w])
                E=[jnp.exp2(z-mx) for z in Z]
                den=E[0]
                for w in range(1,8): den=den+E[w]
                rden=1.0/den
                A=[e*rden for e in E]
                outs=[]
                for j in range(8):
                    o=A[0]*vf_s[j,pl.ds(lb+HALO,R),:]
                    for w in range(1,8): o=o+A[w]*vf_s[j,pl.ds(lb+HALO-2*w,R),:]
                    outs.append(pltpu.bitcast(o.astype(bf16),i32))
                nat=permute(outs,masks)
                for c in range(8):
                    ob_s[pl.ds(b,R),c*128:(c+1)*128]=pltpu.bitcast(nat[c],bf16)

            def body(f,c):
                with sc('itwait'):
                    @pl.when(first)
                    def _():
                        for cp in w13copy(f+1): cp.wait()
                        w2copy(f+1).wait()
                        @pl.when(f+1+AHEAD<=NTRIP)
                        def _():
                            for cp in w13copy(f+1+AHEAD): cp.start()
                            w2copy(f+1+AHEAD).start()
                        @pl.when(f+AHEAD==NTRIP)
                        def _():
                            wocopy().start()
                    @pl.when(jnp.logical_and(f==0,t+1<NT))
                    def _():
                        for p in range(XP): xcopy(t+1,p).wait()
                with sc('itbody'):
                    def att():
                        if mode!='noattn':
                            b0=pl.multiple_of(f*RPT,RPT)
                            perm_kv(b0)
                            for uu in range(RPT//unit):
                                attn(pl.multiple_of(b0+uu*unit,unit),uu*unit)
                            rs=pl.ds(b0,RPT)
                            xn_s[1-slot,rs,:]=layernorm(xb[1-slot,rs,:])
                    if inter:
                        b0=pl.multiple_of(f*RPT,RPT)
                        nu=RPT//unit
                        perm_kv(b0)
                        for k in range(SUB):
                            ffn(pl.ds(pl.multiple_of(FC0+f*FT+k*FC,128),FC),False)
                            for uu in range(k*nu//SUB,(k+1)*nu//SUB):
                                attn(pl.multiple_of(b0+uu*unit,unit),uu*unit)
                        rs=pl.ds(b0,RPT)
                        xn_s[1-slot,rs,:]=layernorm(xb[1-slot,rs,:])
                        return c
                    if att_first: att()
                    for k in range(SUB):
                        ffn(pl.ds(pl.multiple_of(FC0+f*FT+k*FC,128),FC),False)
                    if not att_first: att()
                return c
            jax.lax.fori_loop(0,NTRIP,body,0)
            with sc('wowait'):
                @pl.when(first)
                def _():
                    wocopy().wait()
                @pl.when(t>=2)
                def _():
                    for r in range(OB): ocopy(t-2,r).wait()
            with sc('wo'):
                raw_s[:,0:HALO,:]=raw_s[:,TM:TM+HALO,:]
                for r in range(OB):
                    rs=slice(r*ORB,(r+1)*ORB)
                    ff=acc_s[rs,:]
                    g=silu_f(ff)
                    s=jnp.dot(ob_s[rs,:],wo_s[...],preferred_element_type=f32)
                    ob_out[slot,rs,:]=(xb[slot,rs,:].astype(f32)+s*g).astype(bf16)
                    ocopy(t,r).start()
                @pl.when(t+2<NT)
                def _():
                    for p in range(XP): xcopy(t+2,p).start()
            return carry
        def tile_s(t,c):
            with sc('tile'):
                return tile(t,c)
        jax.lax.fori_loop(0,NT,tile_s,0)
        for t in range(NT-2,NT):
            for r in range(OB): ocopy(t,r).wait()

    anyspec=pl.BlockSpec(memory_space=pl.ANY)
    @jax.jit
    def fn(x,wqkv,wo,bx,w1,w3,w2):
        out=pl.pallas_call(kern,
            in_specs=[anyspec]*6,
            out_specs=anyspec,
            out_shape=jax.ShapeDtypeStruct((S,D),bf16),
            scratch_shapes=[pltpu.VMEM((2,TM,D),bf16),pltpu.VMEM((D,3*D),bf16),pltpu.VMEM((D,D),bf16),
                            pltpu.VMEM((D,F),bf16),pltpu.VMEM((D,F),bf16),pltpu.VMEM((F,D),bf16),
                            pltpu.VMEM((2,TM,D),bf16),
                            pltpu.VMEM((2,TM,D),bf16),pltpu.VMEM((2,TM+HALO,D),bf16),pltpu.VMEM((8,RPT+HALO,128),f32),
                            pltpu.VMEM((8,RPT+HALO,128),f32),pltpu.VMEM((TM,D),bf16),pltpu.VMEM((TM,D),f32),
                            pltpu.SemaphoreType.DMA((2,XP)),pltpu.SemaphoreType.DMA((2,OB)),pltpu.SemaphoreType.DMA((4,)),
                            pltpu.SemaphoreType.DMA((3,NTRIP+1))],
            compiler_params=pltpu.CompilerParams(vmem_limit_bytes=110*2**20))(x[0],wqkv,wo,w1,w3,w2)
        return out[None]
    return fn


_fn = mk(**dict(stage=1,XP=1))


@jax.jit
def pallas_recurrent_scan__sliding_local_dilated__glu_gated_swiglu__prompt_kernel(
    A_x, A_wqkv, A_wo, B_x, B_w1, B_w3, B_w2
):
    return _fn(A_x, A_wqkv, A_wo, B_x, B_w1, B_w3, B_w2)
```

```python
import contextlib
import jax
import jax.numpy as jnp
import numpy as np
from jax.experimental import pallas as pl
from jax.experimental.pallas import tpu as pltpu
S,D,F=2048,1024,3584
f32=jnp.float32; bf16=jnp.bfloat16; i32=jnp.int32
HALO=16

def lane_field_masks(shape):
    lane=jax.lax.broadcasted_iota(i32,shape,len(shape)-1)
    fld=(lane>>1)&7
    return [((fld>>b)&1)==1 for b in range(3)]

FAKE=[0]
def roll(x,k,kind):
    if FAKE[0]&kind: return x+jnp.asarray(k,x.dtype)
    return pltpu.roll(x,k,1)
def permute(cols,masks):
    R=[cols[c] if c==0 else roll(cols[c],2*c,1) for c in range(8)]
    X=[R[(-c)%8] for c in range(8)]
    for b in range(3):
        sh=1<<b
        X=[jnp.where(masks[b],X[(j-sh)%8],X[j]) for j in range(8)]
    return [X[j] if j==0 else roll(X[j],128-2*j,1) for j in range(8)]

def silu_t(g):
    hg=0.5*g
    return hg+hg*jnp.tanh(hg)
def silu_e(g):
    return g*jax.nn.sigmoid(g)
def silu_a(g):
    return g*pl.reciprocal(1.0+jnp.exp(-g),approx=True)
def layernorm(x):
    x=x.astype(f32)
    m=jnp.mean(x,axis=-1,keepdims=True)
    xc=x-m
    var=jnp.mean(xc*xc,axis=-1,keepdims=True)
    return (xc*jax.lax.rsqrt(var+1e-5)).astype(bf16)

def mk(TM=512, FC0=512, NTRIP=4, SUB=2, unit=16, OB=2, mode='full', prof=False, lnrows=None, XP=2, stage=0, att_first=False, AHEAD=2, silu='tanh', inter=False, skipln=False, aligned=False, noroll=False, pad=0, fake=0, qpark=True, u8=0, oreload=False, chain=None, step=1, chainall=0, lnpos='end'):
    FAKE[0]=fake
    FT=(F-FC0)//NTRIP; FC=FT//SUB
    assert FC0+NTRIP*SUB*FC==F and FC%128==0
    RPT=-(-TM//(NTRIP*16))*16
    NT=S//TM
    ORB=TM//OB
    XR=TM//XP
    silu_f={'tanh':silu_t,'exp':silu_e,'approx':silu_a}[silu]
    c_scale=float(32**-0.5*np.log2(np.e))
    sc=lambda n: jax.named_scope(n) if (prof is True or (prof and (n in prof or n.startswith('pro')))) else contextlib.nullcontext()
    def kern(x_hbm,wqkv_hbm,wo_hbm,w1_hbm,w3_hbm,w2_hbm,o_hbm,
             xb,wqkv_s,wo_s,w1_s,w3_s,w2_s,ob_out,xn_s,qraw_s,raw_s,kf_s,vf_s,qf_s,ob_s,acc_s,xsem,osem,wsem,fsem):
        B=lambda v: pltpu.bitcast(v,bf16)
        I=lambda v: pltpu.bitcast(v,i32)
        xb_d,wqkv_d,wo_d,w1_d,w3_d,w2_d,ob_out_d,xn_d,raw_d,ob_d,qraw_d=[r.bitcast(bf16) for r in (xb,wqkv_s,wo_s,w1_s,w3_s,w2_s,ob_out,xn_s,raw_s,ob_s,qraw_s)]
        def xcopy(t,p):
            return pltpu.make_async_copy(x_hbm.at[pl.ds(pl.multiple_of(t*TM+p*XR,XR),XR),:],xb_d.at[t%2,pl.ds(p*XR,XR),:],xsem.at[t%2,p])
        def ocopy(t,r):
            return pltpu.make_async_copy(ob_out_d.at[t%2,pl.ds(r*ORB,ORB),:],o_hbm.at[pl.ds(pl.multiple_of(t*TM+r*ORB,ORB),ORB),:],osem.at[t%2,r])
        def fsl(f):
            if isinstance(f,int):
                return pl.ds(0,FC0) if f==0 else pl.ds(FC0+(f-1)*FT,FT)
            return pl.ds(pl.multiple_of(FC0+(f-1)*FT,128),FT)
        def w13copy(f):
            sl=fsl(f)
            return [pltpu.make_async_copy(w1_hbm.at[:,sl],w1_d.at[:,sl],fsem.at[0,f]),
                    pltpu.make_async_copy(w3_hbm.at[:,sl],w3_d.at[:,sl],fsem.at[1,f])]
        def w2copy(f):
            sl=fsl(f)
            return pltpu.make_async_copy(w2_hbm.at[sl,:],w2_d.at[sl,:],fsem.at[2,f])
        def qkvcopy(p):
            return pltpu.make_async_copy(wqkv_hbm.at[:,pl.ds(p*D,D)],wqkv_d.at[:,pl.ds(p*D,D)],wsem.at[p])
        def wocopy():
            return pltpu.make_async_copy(wo_hbm,wo_d,wsem.at[3])

        with sc('pro_issue'):
            for p in range(XP): xcopy(0,p).start()
            for c in w13copy(0): c.start()
            if stage==1: w2copy(0).start()
            raw_s[:,0:HALO//2,:]=jnp.zeros((2,HALO//2,D),i32)
        for p in range(XP):
            with sc('pro_xwait'):
                xcopy(0,p).wait()
            with sc('pro_ln'):
                xn_d[0,p*XR:(p+1)*XR,:]=layernorm(xb_d[0,p*XR:(p+1)*XR,:])
        with sc('pro_wwait'):
            for c in w13copy(0): c.wait()
            if stage==0: w2copy(0).start()
            qkvcopy(0).start()
            if stage==2:
                w2copy(0).start()

        def tile(t,carry):
            slot=t%2
            first=t==0
            xn_t=xn_d.at[slot]
            def ffn(st,n,init):
                sl=pl.ds(st,n); sl2=pl.ds(st//2 if isinstance(st,int) else pl.multiple_of(st//2,64),n//2)
                g=jnp.dot(xn_t[...],w1_d[:,sl],preferred_element_type=f32)
                u=jnp.dot(xn_t[...],w3_d[:,sl],preferred_element_type=f32)
                h=(silu_f(g)*u).astype(bf16)
                d=jnp.dot(h,w2_d[sl,:],preferred_element_type=f32)
                if init: acc_s[...]=d
                else: acc_s[...]+=d
            with sc('w0wait'):
                @pl.when(first)
                def _():
                    w2copy(0).wait()
                    qkvcopy(1).start(); qkvcopy(2).start()
            with sc('ffn0'):
                ffn(0,FC0,True)
            with sc('qkvwait'):
                @pl.when(first)
                def _():
                    for p in range(3): qkvcopy(p).wait()
                    for p in range(XP): xcopy(1,p).start()
                    for f in range(1,AHEAD+1):
                        for c in w13copy(f): c.start()
                        w2copy(f).start()
            with sc('qkv'):
                for part in range(3):
                    r=jnp.dot(xn_t[...],wqkv_d[:,part*D:(part+1)*D],preferred_element_type=f32).astype(bf16)
                    if part==0: (ob_d if qpark else qraw_d)[...]=r
                    else: raw_d[part-1,HALO:HALO+TM,:]=r

            def perm_kv(b):
                n=(RPT+HALO)
                masks=lane_field_masks((n//2,128))
                for part,dst in ((0,kf_s),(1,vf_s)):
                    ri=raw_s[part,pl.ds(pl.multiple_of(b//2,8),n//2),:]
                    cols=permute([ri[:,c*128:(c+1)*128] for c in range(8)],masks)
                    for j in range(8):
                        dst[j,:,:]=pltpu.bitcast(cols[j],bf16).astype(f32)

            def attn(b,lb,dep=None,zero=None):
                R=unit
                row=jax.lax.broadcasted_iota(i32,(R,128),0)+(t*TM+b)
                lane=jax.lax.broadcasted_iota(i32,(R,128),1)
                b0=(lane&1)==1; b4=(lane&16)!=0
                masks=lane_field_masks((R//2,128))
                qi=(ob_s if qpark else qraw_s)[pl.ds(pl.multiple_of(b//2,8),R//2),:]
                qcols=[qi[:,c*128:(c+1)*128] for c in range(8)]
                if dep is not None:
                    dz=dep&zero
                    if chain[1]=='pre': qcols=[c|dz for c in qcols]
                qc=permute(qcols,masks)
                if dep is not None and chain[1]=='post': qc=[c|dz for c in qc]
                q=[pltpu.bitcast(c,bf16).astype(f32)*c_scale for c in qc]
                Z=[]
                for w in range(8):
                    st=pl.ds(lb+HALO-2*w,R) if not aligned else pl.ds((lb+8*w)%RPT,R)
                    z=q[0]*kf_s[0,st,:]
                    for j in range(1,8): z=z+q[j]*kf_s[j,st,:]
                    if not noroll:
                        z=z+jnp.where(b0,roll(z,1,2),roll(z,127,2))
                        z=z+jnp.where(b4,roll(z,16,2),roll(z,112,2))
                    if w>0: z=jnp.where(row>=2*w,z,-1e9)
                    Z.append(z)
                mx=Z[0]
                for w in range(1,8): mx=jnp.maximum(mx,Z[w])
                E=[jnp.exp2(z-mx) for z in Z]
                den=E[0]
                for w in range(1,8): den=den+E[w]
                rden=1.0/den
                A=[e*rden for e in E]
                outs=[]
                for j in range(8):
                    o=A[0]*vf_s[j,pl.ds(lb+HALO,R),:]
                    for w in range(1,8): o=o+A[w]*vf_s[j,pl.ds(lb+HALO-2*w,R) if not aligned else pl.ds((lb+8*w)%RPT,R),:]
                    if oreload:
                        ob_d[pl.ds(b,R),j*128:(j+1)*128]=o.astype(bf16)
                    else:
                        outs.append(pltpu.bitcast(o.astype(bf16),i32))
                if oreload:
                    oi=ob_s[pl.ds(pl.multiple_of(b//2,8),R//2),:]
                    outs=[oi[:,j*128:(j+1)*128] for j in range(8)]
                nat=permute(outs,masks)
                for c in range(8):
                    ob_s[pl.ds(pl.multiple_of(b//2,8),R//2),c*128:(c+1)*128]=nat[c]
                if chain is None: return None
                if chain[0]=='out': return nat[7][0:8,:]
                if chain[0]=='o': return outs[7][0:8,:]
                if chain[0]=='o3': return outs[3][0:8,:]
                if chain[0]=='rden': return pltpu.bitcast(rden,i32)[0:8,:]
                if chain[0]=='z': return pltpu.bitcast(mx,i32)[0:8,:]
                if chain[0]=='z3': return pltpu.bitcast(Z[3],i32)[0:8,:]

            def perm_kv_rows(b,r0,n,dep,zero):
                masks=lane_field_masks((n//2,128))
                last=None
                for part,dst in ((0,kf_s),(1,vf_s)):
                    ri=raw_s[part,pl.ds(pl.multiple_of((b+r0)//2,8),n//2),:]
                    cs=[ri[:,c*128:(c+1)*128] for c in range(8)]
                    if dep is not None:
                        dz=dep&zero
                        if n>16: dz=jnp.concatenate([dz]*(n//16),axis=0)
                        cs=[c|dz for c in cs]
                    cols=permute(cs,masks)
                    for j in range(8):
                        dst[j,r0:r0+n,:]=pltpu.bitcast(cols[j],bf16).astype(f32)
                    last=cols[7][0:8,:]
                return last
            def ln_rows(b,n,dep,zero):
                rs=pl.ds(pl.multiple_of(b//2,8),n//2)
                xi=xb[1-slot,rs,:]
                if dep is not None:
                    dz=dep&zero
                    xi=xi|jnp.concatenate([dz]*8,axis=1)
                y=layernorm(B(xi))
                xn_d[1-slot,pl.ds(b,n),:]=y
                return pltpu.bitcast(y[:,0:128],i32)
            def perm_q(b):
                masks=lane_field_masks((RPT//2,128))
                qi=(ob_s if qpark else qraw_s)[pl.ds(pl.multiple_of(b//2,8),RPT//2),:]
                qc=permute([qi[:,c*128:(c+1)*128] for c in range(8)],masks)
                for j in range(8):
                    qf_s[j,:,:]=pltpu.bitcast(qc[j],bf16).astype(f32)*c_scale
            def attn8(b,lb,zero):
                R=8
                row=jax.lax.broadcasted_iota(i32,(R,128),0)+(t*TM+b+lb)
                lane=jax.lax.broadcasted_iota(i32,(R,128),1)
                b0=(lane&1)==1; b4=(lane&16)!=0
                qs=pl.ds(pl.multiple_of(lb+zero,8),R)
                q=[qf_s[j,qs,:] for j in range(8)]
                Z=[]
                for w in range(8):
                    st=pl.ds(lb+HALO-2*w,R)
                    z=q[0]*kf_s[0,st,:]
                    for j in range(1,8): z=z+q[j]*kf_s[j,st,:]
                    z=z+jnp.where(b0,roll(z,1,2),roll(z,127,2))
                    z=z+jnp.where(b4,roll(z,16,2),roll(z,112,2))
                    if w>0: z=jnp.where(row>=2*w,z,-1e9)
                    Z.append(z)
                mx=Z[0]
                for w in range(1,8): mx=jnp.maximum(mx,Z[w])
                E=[jnp.exp2(z-mx) for z in Z]
                den=E[0]
                for w in range(1,8): den=den+E[w]
                rden=1.0/den
                A=[e*rden for e in E]
                for j in range(8):
                    o=A[0]*vf_s[j,pl.ds(lb+HALO,R),:]
                    for w in range(1,8): o=o+A[w]*vf_s[j,pl.ds(lb+HALO-2*w,R),:]
                    qf_s[j,qs,:]=o
            def unperm_o(b,r0,n):
                masks=lane_field_masks((n//2,128))
                outs=[pltpu.bitcast(qf_s[j,r0:r0+n,:].astype(bf16),i32) for j in range(8)]
                nat=permute(outs,masks)
                for c in range(8):
                    ob_s[pl.ds(pl.multiple_of((b+r0)//2,8),n//2),c*128:(c+1)*128]=nat[c]

            def body(f,c):
                with sc('itwait'):
                    @pl.when(first)
                    def _():
                        for cp in w13copy(f+1): cp.wait()
                        w2copy(f+1).wait()
                        @pl.when(f+1+AHEAD<=NTRIP)
                        def _():
                            for cp in w13copy(f+1+AHEAD): cp.start()
                            w2copy(f+1+AHEAD).start()
                        @pl.when(f+AHEAD==NTRIP)
                        def _():
                            wocopy().start()
                    @pl.when(jnp.logical_and(f==0,t+1<NT))
                    def _():
                        for p in range(XP): xcopy(t+1,p).wait()
                with sc('itbody'):
                    def att():
                        if chainall:
                            b0=pl.multiple_of(jnp.minimum(f*RPT,TM-RPT),16)
                            zero=jnp.full((8,128),jnp.minimum(f,0),i32)
                            dep=None
                            for uu in range(RPT//unit):
                                bu=pl.multiple_of(b0+uu*unit,unit)
                                if uu==0: dep=perm_kv_rows(b0,0,HALO+unit,dep,zero)
                                else: dep=perm_kv_rows(b0,HALO+uu*unit,unit,dep,zero)
                                if chainall==2: dep=None if uu==0 else d_prev
                                d_prev=dep=attn(bu,uu*unit,dep,zero)
                                dl=ln_rows(bu,unit,dep,zero)
                                if chainall!=3: dep=dl
                            return
                        b0=pl.multiple_of(jnp.minimum(f*RPT,TM-RPT),16)
                        if mode in('full','perm','permattn'): perm_kv(b0)
                        if u8:
                            zero=jnp.minimum(f,0)
                            perm_q(b0)
                            for uu in range(RPT//8):
                                attn8(b0,uu*8,zero if u8==1 or (u8==2 and uu%2==0) else 0)
                                if uu%2==1: unperm_o(b0,(uu-1)*8,16)
                        elif mode in('full','attn','permattn'):
                            zero=jnp.full((8,128),jnp.minimum(f,0),i32)
                            deps=[]
                            for uu in range(RPT//unit):
                                dp=deps[uu-step] if (chain is not None and uu>=step) else None
                                deps.append(attn(pl.multiple_of(b0+uu*unit,unit),uu*unit,dp,zero))
                        if mode in('full','ln'):
                            rs=pl.ds(b0,RPT)
                            xn_d[1-slot,rs,:]=layernorm(xb_d[1-slot,rs,:])
                    if inter:
                        b0=pl.multiple_of(jnp.minimum(f*RPT,TM-RPT),16)
                        nu=RPT//unit
                        perm_kv(b0)
                        for k in range(SUB):
                            ffn(pl.multiple_of(FC0+f*FT+k*FC,128),FC,False)
                            for uu in range(k*nu//SUB,(k+1)*nu//SUB):
                                attn(pl.multiple_of(b0+uu*unit,unit),uu*unit)
                        rs=pl.ds(b0,RPT)
                        xn_d[1-slot,rs,:]=layernorm(xb_d[1-slot,rs,:])
                        return c
                    if att_first: att()
                    for k in range(SUB):
                        ffn(pl.multiple_of(FC0+f*FT+k*FC,128),FC,False)
                    if not att_first: att()
                return c
            jax.lax.fori_loop(0,NTRIP,body,0)
            with sc('wowait'):
                @pl.when(first)
                def _():
                    wocopy().wait()
                @pl.when(t>=2)
                def _():
                    for r in range(OB): ocopy(t-2,r).wait()
            with sc('wo'):
                raw_s[:,0:HALO//2,:]=raw_s[:,TM//2:(TM+HALO)//2,:]
                for pp in range(pad):
                    pass
                for r in range(OB):
                    rs=slice(r*ORB,(r+1)*ORB)
                    ff=acc_s[rs,:]
                    g=silu_f(ff)
                    r2=slice(r*ORB//2,(r+1)*ORB//2)
                    s=jnp.dot(ob_d[rs,:],wo_d[...],preferred_element_type=f32)
                    ob_out_d[slot,rs,:]=(xb_d[slot,rs,:].astype(f32)+s*g).astype(bf16)
                    ocopy(t,r).start()
                @pl.when(t+2<NT)
                def _():
                    for p in range(XP): xcopy(t+2,p).start()
            return carry
        def tile_s(t,c):
            with sc('tile'):
                return tile(t,c)
        jax.lax.fori_loop(0,NT,tile_s,0)
        for t in range(NT-2,NT):
            for r in range(OB): ocopy(t,r).wait()

    anyspec=pl.BlockSpec(memory_space=pl.ANY)
    @jax.jit
    def fn(x,wqkv,wo,bx,w1,w3,w2):
        out=pl.pallas_call(kern,
            in_specs=[anyspec]*6,
            out_specs=anyspec,
            out_shape=jax.ShapeDtypeStruct((S,D),bf16),
            scratch_shapes=[pltpu.VMEM((2,TM//2,D),i32),pltpu.VMEM((D//2,3*D),i32),pltpu.VMEM((D//2,D),i32),
                            pltpu.VMEM((D//2,F),i32),pltpu.VMEM((D//2,F),i32),pltpu.VMEM((F//2,D),i32),
                            pltpu.VMEM((2,TM//2,D),i32),
                            pltpu.VMEM((2,TM//2,D),i32),pltpu.VMEM((TM//2,D),i32),pltpu.VMEM((2,(TM+HALO)//2,D),i32),pltpu.VMEM((8,RPT+HALO,128),f32),
                            pltpu.VMEM((8,RPT+HALO,128),f32),pltpu.VMEM((8,RPT,128),f32),pltpu.VMEM((TM//2,D),i32),pltpu.VMEM((TM,D),f32),
                            pltpu.SemaphoreType.DMA((2,XP)),pltpu.SemaphoreType.DMA((2,OB)),pltpu.SemaphoreType.DMA((4,)),
                            pltpu.SemaphoreType.DMA((3,NTRIP+1))],
            compiler_params=pltpu.CompilerParams(vmem_limit_bytes=110*2**20))(x[0],wqkv,wo,w1,w3,w2)
        return out[None]
    return fn


_fn = mk(**dict(stage=1,XP=1,qpark=False,chain=('rden','post'),chainall=3))


@jax.jit
def pallas_recurrent_scan__sliding_local_dilated__glu_gated_swiglu__prompt_kernel(
    A_x, A_wqkv, A_wo, B_x, B_w1, B_w3, B_w2
):
    return _fn(A_x, A_wqkv, A_wo, B_x, B_w1, B_w3, B_w2)
```

```python
import contextlib
import jax
import jax.numpy as jnp
import numpy as np
from jax.experimental import pallas as pl
from jax.experimental.pallas import tpu as pltpu
S,D,F=2048,1024,3584
f32=jnp.float32; bf16=jnp.bfloat16; i32=jnp.int32
HALO=16

def lane_field_masks(shape):
    lane=jax.lax.broadcasted_iota(i32,shape,len(shape)-1)
    fld=(lane>>1)&7
    return [((fld>>b)&1)==1 for b in range(3)]

FAKE=[0]
def roll(x,k,kind):
    if FAKE[0]&kind: return x+jnp.asarray(k,x.dtype)
    return pltpu.roll(x,k,1)
def permute(cols,masks):
    R=[cols[c] if c==0 else roll(cols[c],2*c,1) for c in range(8)]
    X=[R[(-c)%8] for c in range(8)]
    for b in range(3):
        sh=1<<b
        X=[jnp.where(masks[b],X[(j-sh)%8],X[j]) for j in range(8)]
    return [X[j] if j==0 else roll(X[j],128-2*j,1) for j in range(8)]

def silu_t(g):
    hg=0.5*g
    return hg+hg*jnp.tanh(hg)
def silu_e(g):
    return g*jax.nn.sigmoid(g)
def silu_a(g):
    return g*pl.reciprocal(1.0+jnp.exp(-g),approx=True)
def layernorm(x):
    x=x.astype(f32)
    m=jnp.mean(x,axis=-1,keepdims=True)
    xc=x-m
    var=jnp.mean(xc*xc,axis=-1,keepdims=True)
    return (xc*jax.lax.rsqrt(var+1e-5)).astype(bf16)

def mk(TM=512, FC0=512, NTRIP=4, SUB=2, unit=16, OB=2, mode='full', prof=False, lnrows=None, XP=2, stage=0, att_first=False, AHEAD=2, silu='tanh', inter=False, skipln=False, aligned=False, noroll=False, pad=0, fake=0, qpark=True, u8=0, oreload=False, chain=None, step=1, chainall=0, PF=128, PQ=512, PA=2, LNR=128, lnpos='end'):
    FAKE[0]=fake
    FT=(F-FC0)//NTRIP; FC=FT//SUB
    assert FC0+NTRIP*SUB*FC==F and FC%128==0
    RPT=-(-TM//(NTRIP*16))*16
    NT=S//TM
    ORB=TM//OB
    XR=TM//XP
    silu_f={'tanh':silu_t,'exp':silu_e,'approx':silu_a}[silu]
    c_scale=float(32**-0.5*np.log2(np.e))
    sc=lambda n: jax.named_scope(n) if (prof is True or (prof and (n in prof or n.startswith('pro')))) else contextlib.nullcontext()
    def kern(x_hbm,wqkv_hbm,wo_hbm,w1_hbm,w3_hbm,w2_hbm,o_hbm,
             xb,wqkv_s,wo_s,w1_s,w3_s,w2_s,ob_out,xn_s,raw_s,kf_s,vf_s,qf_s,ob_s,acc_s,xsem,osem,wsem,fsem,psem,qsem):
        B=lambda v: pltpu.bitcast(v,bf16)
        I=lambda v: pltpu.bitcast(v,i32)
        xb_d,wqkv_d,wo_d,w1_d,w3_d,w2_d,ob_out_d,xn_d,raw_d,ob_d=[r.bitcast(bf16) for r in (xb,wqkv_s,wo_s,w1_s,w3_s,w2_s,ob_out,xn_s,raw_s,ob_s)]
        def xcopy(t,p):
            return pltpu.make_async_copy(x_hbm.at[pl.ds(pl.multiple_of(t*TM+p*XR,XR),XR),:],xb_d.at[t%2,pl.ds(p*XR,XR),:],xsem.at[t%2,p])
        def ocopy(t,r):
            return pltpu.make_async_copy(ob_out_d.at[t%2,pl.ds(r*ORB,ORB),:],o_hbm.at[pl.ds(pl.multiple_of(t*TM+r*ORB,ORB),ORB),:],osem.at[t%2,r])
        def fsl(f):
            if isinstance(f,int):
                return pl.ds(0,FC0) if f==0 else pl.ds(FC0+(f-1)*FT,FT)
            return pl.ds(pl.multiple_of(FC0+(f-1)*FT,128),FT)
        def w13copy(f):
            sl=fsl(f)
            return [pltpu.make_async_copy(w1_hbm.at[:,sl],w1_d.at[:,sl],fsem.at[0,f]),
                    pltpu.make_async_copy(w3_hbm.at[:,sl],w3_d.at[:,sl],fsem.at[1,f])]
        def w2copy(f):
            sl=fsl(f)
            return pltpu.make_async_copy(w2_hbm.at[sl,:],w2_d.at[sl,:],fsem.at[2,f])
        def qkvcopy(p):
            return pltpu.make_async_copy(wqkv_hbm.at[:,pl.ds(p*D,D)],wqkv_d.at[:,pl.ds(p*D,D)],wsem.at[p])
        def wocopy():
            return pltpu.make_async_copy(wo_hbm,wo_d,wsem.at[3])

        NP=FC0//PF; NQ=3*D//PQ
        def pcopy(i):
            sl=pl.ds(pl.multiple_of(i*PF,PF),PF)
            return [pltpu.make_async_copy(w1_hbm.at[:,sl],w1_d.at[:,sl],psem.at[0,i]),
                    pltpu.make_async_copy(w3_hbm.at[:,sl],w3_d.at[:,sl],psem.at[1,i]),
                    pltpu.make_async_copy(w2_hbm.at[sl,:],w2_d.at[sl,:],psem.at[2,i])]
        def qcopy(i):
            sl=pl.ds(pl.multiple_of(i*PQ,PQ),PQ)
            return pltpu.make_async_copy(wqkv_hbm.at[:,sl],wqkv_d.at[:,sl],qsem.at[i])
        def trip_start(f):
            for cp in w13copy(f): cp.start()
            w2copy(f).start()
        def ffn_g(xn,st,n,init):
            sl=pl.ds(st,n)
            g=jnp.dot(xn[...],w1_d[:,sl],preferred_element_type=f32)
            u=jnp.dot(xn[...],w3_d[:,sl],preferred_element_type=f32)
            h=(silu_f(g)*u).astype(bf16)
            d=jnp.dot(h,w2_d[sl,:],preferred_element_type=f32)
            if init is True: acc_s[...]=d
            elif init is False: acc_s[...]+=d
            else: acc_s[...]=jnp.where(init,0.0,acc_s[...])+d
        def start_piece(g):
            if g<NP:
                for c in pcopy(g): c.start()
            elif g<NP+NQ: qcopy(g-NP).start()
            elif g==NP+NQ:
                for p in range(XP): xcopy(1,p).start()
                trip_start(1)
            elif g==NP+NQ+1: trip_start(2)
        def start_piece_dyn(g,lo,hi):
            if lo<NP:
                @pl.when(g<NP)
                def _():
                    for c in pcopy(g): c.start()
            if lo<NP+NQ and hi>NP:
                @pl.when(jnp.logical_and(g>=NP,g<NP+NQ))
                def _():
                    qcopy(g-NP).start()
            for gs in (NP+NQ,NP+NQ+1):
                if lo<=gs<hi:
                    @pl.when(g==gs)
                    def _():
                        start_piece(gs)
        with sc('pro_issue'):
            for p in range(XP): xcopy(0,p).start()
            for g in range(PA): start_piece(g)
            raw_s[1:3,0:HALO//2,:]=jnp.zeros((2,HALO//2,D),i32)
            def zacc(i,c):
                acc_s[pl.ds(pl.multiple_of(i*64,64),64),:]=jnp.zeros((64,D),f32)
                return c
            jax.lax.fori_loop(0,TM//64,zacc,0)
        def pro_ln(p,c):
            with sc('pro_xwait'):
                xcopy(0,p).wait()
            with sc('pro_ln'):
                def lnb(i,c2):
                    rs=pl.ds(pl.multiple_of(p*XR+i*LNR,LNR),LNR)
                    xn_d[0,rs,:]=layernorm(xb_d[0,rs,:])
                    return c2
                jax.lax.fori_loop(0,XR//LNR,lnb,0)
            return c
        jax.lax.fori_loop(0,XP,pro_ln,0)
        def pro_ffn(i,c):
            for cp in pcopy(i): cp.wait()
            start_piece_dyn(i+PA,PA,NP+PA)
            with sc('pro_ffn'):
                ffn_g(xn_d.at[0],pl.multiple_of(i*PF,PF),PF,False)
            return c
        jax.lax.fori_loop(0,NP,pro_ffn,0)
        def pro_qkv(i,c):
            qcopy(i).wait()
            start_piece_dyn(NP+i+PA,NP+PA,NP+NQ+PA)
            with sc('pro_qkv'):
                cs=pl.ds(pl.multiple_of(i*PQ,PQ),PQ)
                r=jnp.dot(xn_d[0],wqkv_d[:,cs],preferred_element_type=f32).astype(bf16)
                part=(i*PQ)//D
                cs2=pl.ds(pl.multiple_of((i*PQ)%D,PQ),PQ)
                raw_d[part,HALO:HALO+TM,cs2]=r
            return c
        jax.lax.fori_loop(0,NQ,pro_qkv,0)
        for g in range(NP+NQ+PA,NP+NQ+2): start_piece(g)

        def tile(t,carry):
            slot=t%2
            first=t==0
            xn_t=xn_d.at[slot]
            def front(tn):
                xn_n=xn_d.at[tn%2]
                ffn_g(xn_n,0,FC0,True)
                for part in range(3):
                    r=jnp.dot(xn_n[...],wqkv_d[:,part*D:(part+1)*D],preferred_element_type=f32).astype(bf16)
                    raw_d[part,HALO:HALO+TM,:]=r
            ffn=lambda st,n,init: ffn_g(xn_t,st,n,init)

            def perm_kv(b):
                n=(RPT+HALO)
                masks=lane_field_masks((n//2,128))
                for part,dst in ((1,kf_s),(2,vf_s)):
                    ri=raw_s[part,pl.ds(pl.multiple_of(b//2,8),n//2),:]
                    cols=permute([ri[:,c*128:(c+1)*128] for c in range(8)],masks)
                    for j in range(8):
                        dst[j,:,:]=pltpu.bitcast(cols[j],bf16).astype(f32)

            def attn(b,lb,dep=None,zero=None):
                R=unit
                row=jax.lax.broadcasted_iota(i32,(R,128),0)+(t*TM+b)
                lane=jax.lax.broadcasted_iota(i32,(R,128),1)
                b0=(lane&1)==1; b4=(lane&16)!=0
                masks=lane_field_masks((R//2,128))
                qi=raw_s[0,pl.ds(pl.multiple_of((b+HALO)//2,8),R//2),:]
                qcols=[qi[:,c*128:(c+1)*128] for c in range(8)]
                if dep is not None:
                    dz=dep&zero
                    if chain[1]=='pre': qcols=[c|dz for c in qcols]
                qc=permute(qcols,masks)
                if dep is not None and chain[1]=='post': qc=[c|dz for c in qc]
                q=[pltpu.bitcast(c,bf16).astype(f32)*c_scale for c in qc]
                Z=[]
                for w in range(8):
                    st=pl.ds(lb+HALO-2*w,R) if not aligned else pl.ds((lb+8*w)%RPT,R)
                    z=q[0]*kf_s[0,st,:]
                    for j in range(1,8): z=z+q[j]*kf_s[j,st,:]
                    if not noroll:
                        z=z+jnp.where(b0,roll(z,1,2),roll(z,127,2))
                        z=z+jnp.where(b4,roll(z,16,2),roll(z,112,2))
                    if w>0: z=jnp.where(row>=2*w,z,-1e9)
                    Z.append(z)
                mx=Z[0]
                for w in range(1,8): mx=jnp.maximum(mx,Z[w])
                E=[jnp.exp2(z-mx) for z in Z]
                den=E[0]
                for w in range(1,8): den=den+E[w]
                rden=1.0/den
                A=[e*rden for e in E]
                outs=[]
                for j in range(8):
                    o=A[0]*vf_s[j,pl.ds(lb+HALO,R),:]
                    for w in range(1,8): o=o+A[w]*vf_s[j,pl.ds(lb+HALO-2*w,R) if not aligned else pl.ds((lb+8*w)%RPT,R),:]
                    if oreload:
                        ob_d[pl.ds(b,R),j*128:(j+1)*128]=o.astype(bf16)
                    else:
                        outs.append(pltpu.bitcast(o.astype(bf16),i32))
                if oreload:
                    oi=ob_s[pl.ds(pl.multiple_of(b//2,8),R//2),:]
                    outs=[oi[:,j*128:(j+1)*128] for j in range(8)]
                nat=permute(outs,masks)
                for c in range(8):
                    ob_s[pl.ds(pl.multiple_of(b//2,8),R//2),c*128:(c+1)*128]=nat[c]
                if chain is None: return None
                if chain[0]=='out': return nat[7][0:8,:]
                if chain[0]=='o': return outs[7][0:8,:]
                if chain[0]=='o3': return outs[3][0:8,:]
                if chain[0]=='rden': return pltpu.bitcast(rden,i32)[0:8,:]
                if chain[0]=='z': return pltpu.bitcast(mx,i32)[0:8,:]
                if chain[0]=='z3': return pltpu.bitcast(Z[3],i32)[0:8,:]

            def perm_kv_rows(b,r0,n,dep,zero):
                masks=lane_field_masks((n//2,128))
                last=None
                for part,dst in ((1,kf_s),(2,vf_s)):
                    ri=raw_s[part,pl.ds(pl.multiple_of((b+r0)//2,8),n//2),:]
                    cs=[ri[:,c*128:(c+1)*128] for c in range(8)]
                    if dep is not None:
                        dz=dep&zero
                        if n>16: dz=jnp.concatenate([dz]*(n//16),axis=0)
                        cs=[c|dz for c in cs]
                    cols=permute(cs,masks)
                    for j in range(8):
                        dst[j,r0:r0+n,:]=pltpu.bitcast(cols[j],bf16).astype(f32)
                    last=cols[7][0:8,:]
                return last
            def ln_rows(b,n,dep,zero):
                rs=pl.ds(pl.multiple_of(b//2,8),n//2)
                xi=xb[1-slot,rs,:]
                if dep is not None:
                    dz=dep&zero
                    xi=xi|jnp.concatenate([dz]*8,axis=1)
                y=layernorm(B(xi))
                xn_d[1-slot,pl.ds(b,n),:]=y
                return pltpu.bitcast(y[:,0:128],i32)
            def perm_q(b):
                masks=lane_field_masks((RPT//2,128))
                qi=(ob_s if qpark else qraw_s)[pl.ds(pl.multiple_of(b//2,8),RPT//2),:]
                qc=permute([qi[:,c*128:(c+1)*128] for c in range(8)],masks)
                for j in range(8):
                    qf_s[j,:,:]=pltpu.bitcast(qc[j],bf16).astype(f32)*c_scale
            def attn8(b,lb,zero):
                R=8
                row=jax.lax.broadcasted_iota(i32,(R,128),0)+(t*TM+b+lb)
                lane=jax.lax.broadcasted_iota(i32,(R,128),1)
                b0=(lane&1)==1; b4=(lane&16)!=0
                qs=pl.ds(pl.multiple_of(lb+zero,8),R)
                q=[qf_s[j,qs,:] for j in range(8)]
                Z=[]
                for w in range(8):
                    st=pl.ds(lb+HALO-2*w,R)
                    z=q[0]*kf_s[0,st,:]
                    for j in range(1,8): z=z+q[j]*kf_s[j,st,:]
                    z=z+jnp.where(b0,roll(z,1,2),roll(z,127,2))
                    z=z+jnp.where(b4,roll(z,16,2),roll(z,112,2))
                    if w>0: z=jnp.where(row>=2*w,z,-1e9)
                    Z.append(z)
                mx=Z[0]
                for w in range(1,8): mx=jnp.maximum(mx,Z[w])
                E=[jnp.exp2(z-mx) for z in Z]
                den=E[0]
                for w in range(1,8): den=den+E[w]
                rden=1.0/den
                A=[e*rden for e in E]
                for j in range(8):
                    o=A[0]*vf_s[j,pl.ds(lb+HALO,R),:]
                    for w in range(1,8): o=o+A[w]*vf_s[j,pl.ds(lb+HALO-2*w,R),:]
                    qf_s[j,qs,:]=o
            def unperm_o(b,r0,n):
                masks=lane_field_masks((n//2,128))
                outs=[pltpu.bitcast(qf_s[j,r0:r0+n,:].astype(bf16),i32) for j in range(8)]
                nat=permute(outs,masks)
                for c in range(8):
                    ob_s[pl.ds(pl.multiple_of((b+r0)//2,8),n//2),c*128:(c+1)*128]=nat[c]

            def body(f,c):
                with sc('itwait'):
                    @pl.when(first)
                    def _():
                        for cp in w13copy(f+1): cp.wait()
                        w2copy(f+1).wait()
                        @pl.when(f+3<=NTRIP)
                        def _():
                            trip_start(f+3)
                        @pl.when(f+3==NTRIP+1)
                        def _():
                            wocopy().start()
                    @pl.when(jnp.logical_and(f==0,t+1<NT))
                    def _():
                        for p in range(XP): xcopy(t+1,p).wait()
                with sc('itbody'):
                    def att():
                        if chainall:
                            b0=pl.multiple_of(jnp.minimum(f*RPT,TM-RPT),16)
                            zero=jnp.full((8,128),jnp.minimum(f,0),i32)
                            dep=None
                            for uu in range(RPT//unit):
                                bu=pl.multiple_of(b0+uu*unit,unit)
                                if uu==0: dep=perm_kv_rows(b0,0,HALO+unit,dep,zero)
                                else: dep=perm_kv_rows(b0,HALO+uu*unit,unit,dep,zero)
                                if chainall==2: dep=None if uu==0 else d_prev
                                d_prev=dep=attn(bu,uu*unit,dep,zero)
                                dl=ln_rows(bu,unit,dep,zero)
                                if chainall!=3: dep=dl
                            return
                        b0=pl.multiple_of(jnp.minimum(f*RPT,TM-RPT),16)
                        if mode in('full','perm','permattn'): perm_kv(b0)
                        if u8:
                            zero=jnp.minimum(f,0)
                            perm_q(b0)
                            for uu in range(RPT//8):
                                attn8(b0,uu*8,zero if u8==1 or (u8==2 and uu%2==0) else 0)
                                if uu%2==1: unperm_o(b0,(uu-1)*8,16)
                        elif mode in('full','attn','permattn'):
                            zero=jnp.full((8,128),jnp.minimum(f,0),i32)
                            deps=[]
                            for uu in range(RPT//unit):
                                dp=deps[uu-step] if (chain is not None and uu>=step) else None
                                deps.append(attn(pl.multiple_of(b0+uu*unit,unit),uu*unit,dp,zero))
                        if mode in('full','ln'):
                            rs=pl.ds(b0,RPT)
                            xn_d[1-slot,rs,:]=layernorm(xb_d[1-slot,rs,:])
                    if inter:
                        b0=pl.multiple_of(jnp.minimum(f*RPT,TM-RPT),16)
                        nu=RPT//unit
                        perm_kv(b0)
                        for k in range(SUB):
                            ffn(pl.multiple_of(FC0+f*FT+k*FC,128),FC,False)
                            for uu in range(k*nu//SUB,(k+1)*nu//SUB):
                                attn(pl.multiple_of(b0+uu*unit,unit),uu*unit)
                        rs=pl.ds(b0,RPT)
                        xn_d[1-slot,rs,:]=layernorm(xb_d[1-slot,rs,:])
                        return c
                    if att_first: att()
                    for k in range(SUB):
                        ffn(pl.multiple_of(FC0+f*FT+k*FC,128),FC,False)
                    if not att_first: att()
                return c
            jax.lax.fori_loop(0,NTRIP,body,0)
            with sc('wowait'):
                @pl.when(first)
                def _():
                    wocopy().wait()
                @pl.when(t>=2)
                def _():
                    for r in range(OB): ocopy(t-2,r).wait()
            with sc('wo'):
                raw_s[1:3,0:HALO//2,:]=raw_s[1:3,TM//2:(TM+HALO)//2,:]
                for pp in range(pad):
                    pass
                for r in range(OB):
                    rs=slice(r*ORB,(r+1)*ORB)
                    ff=acc_s[rs,:]
                    g=silu_f(ff)
                    r2=slice(r*ORB//2,(r+1)*ORB//2)
                    s=jnp.dot(ob_d[rs,:],wo_d[...],preferred_element_type=f32)
                    ob_out_d[slot,rs,:]=(xb_d[slot,rs,:].astype(f32)+s*g).astype(bf16)
                    ocopy(t,r).start()
                @pl.when(t+2<NT)
                def _():
                    for p in range(XP): xcopy(t+2,p).start()
            with sc('front'):
                @pl.when(t+1<NT)
                def _():
                    front(t+1)
            return carry
        def tile_s(t,c):
            with sc('tile'):
                return tile(t,c)
        jax.lax.fori_loop(0,NT,tile_s,0)
        for t in range(NT-2,NT):
            for r in range(OB): ocopy(t,r).wait()

    anyspec=pl.BlockSpec(memory_space=pl.ANY)
    @jax.jit
    def fn(x,wqkv,wo,bx,w1,w3,w2):
        out=pl.pallas_call(kern,
            in_specs=[anyspec]*6,
            out_specs=anyspec,
            out_shape=jax.ShapeDtypeStruct((S,D),bf16),
            scratch_shapes=[pltpu.VMEM((2,TM//2,D),i32),pltpu.VMEM((D//2,3*D),i32),pltpu.VMEM((D//2,D),i32),
                            pltpu.VMEM((D//2,F),i32),pltpu.VMEM((D//2,F),i32),pltpu.VMEM((F//2,D),i32),
                            pltpu.VMEM((2,TM//2,D),i32),
                            pltpu.VMEM((2,TM//2,D),i32),pltpu.VMEM((3,(TM+HALO)//2,D),i32),pltpu.VMEM((8,RPT+HALO,128),f32),
                            pltpu.VMEM((8,RPT+HALO,128),f32),pltpu.VMEM((8,RPT,128),f32),pltpu.VMEM((TM//2,D),i32),pltpu.VMEM((TM,D),f32),
                            pltpu.SemaphoreType.DMA((2,XP)),pltpu.SemaphoreType.DMA((2,OB)),pltpu.SemaphoreType.DMA((4,)),
                            pltpu.SemaphoreType.DMA((3,NTRIP+1)),pltpu.SemaphoreType.DMA((3,FC0//PF)),pltpu.SemaphoreType.DMA((3*D//PQ,))],
            compiler_params=pltpu.CompilerParams(vmem_limit_bytes=110*2**20))(x[0],wqkv,wo,w1,w3,w2)
        return out[None]
    return fn


_fn = mk(**dict(XP=2,chain=('rden','post'),chainall=3,PA=12))


@jax.jit
def pallas_recurrent_scan__sliding_local_dilated__glu_gated_swiglu__prompt_kernel(
    A_x, A_wqkv, A_wo, B_x, B_w1, B_w3, B_w2
):
    return _fn(A_x, A_wqkv, A_wo, B_x, B_w1, B_w3, B_w2)
```

```python
import contextlib
import jax
import jax.numpy as jnp
import numpy as np
from jax.experimental import pallas as pl
from jax.experimental.pallas import tpu as pltpu

S, D, F = 2048, 1024, 3584
f32, bf16, i32 = jnp.float32, jnp.bfloat16, jnp.int32
HALO = 16
WIN, DIL = 8, 2


def _field_masks(shape):
    lane = jax.lax.broadcasted_iota(i32, shape, len(shape) - 1)
    fld = (lane >> 1) & 7
    return [((fld >> b) & 1) == 1 for b in range(3)]


def _permute(cols, masks):
    r = [cols[c] if c == 0 else pltpu.roll(cols[c], 2 * c, 1) for c in range(8)]
    x = [r[(-c) % 8] for c in range(8)]
    for b in range(3):
        x = [jnp.where(masks[b], x[(j - (1 << b)) % 8], x[j]) for j in range(8)]
    return [x[j] if j == 0 else pltpu.roll(x[j], 128 - 2 * j, 1) for j in range(8)]


def _silu(g):
    hg = 0.5 * g
    return hg + hg * jnp.tanh(hg)


def _layernorm(x):
    x = x.astype(f32)
    m = jnp.mean(x, axis=-1, keepdims=True)
    xc = x - m
    var = jnp.mean(xc * xc, axis=-1, keepdims=True)
    return (xc * jax.lax.rsqrt(var + 1e-5)).astype(bf16)


def mk(TM=512, FC0=512, NTRIP=4, SUB=2, PF=128, PQ=768, OBS=(384, 128), LNR=128, link='rden', early=1, prof=False,
       trip_wait=1, XP=2, var=0, bv=0, zv=0, tok=0, andin=0, slotv=0, kvord=0, qdep=0):
    UNIT = 16
    FT = (F - FC0) // NTRIP
    FC = FT // SUB
    RPT = TM // NTRIP
    NT = S // TM
    NP, NQ = FC0 // PF, 3 * D // PQ
    OST = [sum(OBS[:r]) for r in range(len(OBS))]
    XR = TM // XP
    assert FC0 + NTRIP * SUB * FC == F and FC % 128 == 0 and RPT % UNIT == 0 and sum(OBS) == TM
    c_scale = float((D // 32) ** 0 * 32 ** -0.5 * np.log2(np.e))
    sc = lambda n: (jax.named_scope(n) if (prof is True or (prof and (n in prof or n.startswith('pro'))))
                    else contextlib.nullcontext())

    def kern(x_hbm, wqkv_hbm, wo_hbm, w1_hbm, w3_hbm, w2_hbm, o_hbm,
             xb, wqkv_s, wo_s, w1_s, w3_s, w2_s, out_s, xn_s, raw_s, kf_s, vf_s, ob_s, acc_s,
             x0sem, xsem, osem, psem, qsem, tsem):
        xb_d, wqkv_d, wo_d, w1_d, w3_d, w2_d, out_d, xn_d, raw_d, ob_d = [
            r.bitcast(bf16) for r in (xb, wqkv_s, wo_s, w1_s, w3_s, w2_s, out_s, xn_s, raw_s, ob_s)]

        def x0copy(p):
            rs = pl.ds(pl.multiple_of(p * XR, XR), XR)
            return pltpu.make_async_copy(x_hbm.at[rs, :], xb_d.at[0, rs, :], x0sem.at[p])

        def xcopy(t):
            return pltpu.make_async_copy(x_hbm.at[pl.ds(pl.multiple_of(t * TM, TM), TM), :],
                                         xb_d.at[t & 1], xsem.at[t & 1])

        def ocopy(t, r):
            return pltpu.make_async_copy(out_d.at[t & 1, pl.ds(OST[r], OBS[r]), :],
                                         o_hbm.at[pl.ds(pl.multiple_of(t * TM + OST[r], 16), OBS[r]), :],
                                         osem.at[t & 1, r])

        def fcopies(start, n, sems, i):
            sl = pl.ds(start, n)
            return [pltpu.make_async_copy(w1_hbm.at[:, sl], w1_d.at[:, sl], sems.at[0, i]),
                    pltpu.make_async_copy(w3_hbm.at[:, sl], w3_d.at[:, sl], sems.at[1, i]),
                    pltpu.make_async_copy(w2_hbm.at[sl, :], w2_d.at[sl, :], sems.at[2, i])]

        pcopies = lambda i: fcopies(pl.multiple_of(i * PF, PF), PF, psem, i)
        tcopies = lambda f: fcopies(pl.multiple_of(FC0 + f * FT, 128), FT, tsem, f)

        def qcopy(i):
            sl = pl.ds(pl.multiple_of(i * PQ, 128), PQ)
            return pltpu.make_async_copy(wqkv_hbm.at[:, sl], wqkv_d.at[:, sl], qsem.at[i])

        def wocopy():
            return pltpu.make_async_copy(wo_hbm, wo_d, tsem.at[0, NTRIP])

        def ffn(xn, start, n, init):
            sl = pl.ds(start, n)
            g = jnp.dot(xn[...], w1_d[:, sl], preferred_element_type=f32)
            u = jnp.dot(xn[...], w3_d[:, sl], preferred_element_type=f32)
            h = (_silu(g) * u).astype(bf16)
            d = jnp.dot(h, w2_d[sl, :], preferred_element_type=f32)
            if init:
                acc_s[...] = d
            else:
                acc_s[...] += d

        def late_starts(k):
            if k == 0:
                xcopy(1).start()
                for c in tcopies(0) + tcopies(1): c.start()
            elif k == 1:
                for f in range(2, NTRIP):
                    for c in tcopies(f): c.start()
                wocopy().start()

        with sc('pro_issue'):
            for p in range(XP): x0copy(p).start()
            for i in range(NP):
                for c in pcopies(i): c.start()
            for i in range(NQ): qcopy(i).start()
            for k in range(early): late_starts(k)
            raw_s[0:HALO // 2, D:3 * D] = jnp.zeros((HALO // 2, 2 * D), i32)

            def zero_acc(i, c):
                acc_s[pl.ds(pl.multiple_of(i * 64, 64), 64), :] = jnp.zeros((64, D), f32)
                return c
            jax.lax.fori_loop(0, TM // 64, zero_acc, 0)

        def pro_ln(p, c):
            with sc('pro_xwait'):
                x0copy(p).wait()
            with sc('pro_ln'):
                def rows(i, c2):
                    rs = pl.ds(pl.multiple_of(p * XR + i * LNR, LNR), LNR)
                    xn_d[0, rs, :] = _layernorm(xb_d[0, rs, :])
                    return c2
                jax.lax.fori_loop(0, XR // LNR, rows, 0)
            return c
        jax.lax.fori_loop(0, XP, pro_ln, 0)

        def pro_ffn(i, c):
            for cp in pcopies(i): cp.wait()
            with sc('pro_ffn'):
                ffn(xn_d.at[0], pl.multiple_of(i * PF, PF), PF, False)
            return c
        jax.lax.fori_loop(0, NP, pro_ffn, 0)
        for k in range(early, 2): late_starts(k)

        def pro_qkv(i, c):
            qcopy(i).wait()
            with sc('pro_qkv'):
                cs = pl.ds(pl.multiple_of(i * PQ, 128), PQ)
                r = jnp.dot(xn_d[0], wqkv_d[:, cs], preferred_element_type=f32)
                raw_d[HALO:HALO + TM, cs] = r.astype(bf16)
            return c
        jax.lax.fori_loop(0, NQ, pro_qkv, 0)

        def tile(t, carry):
            slot = (t & 1) if slotv == 0 else t % 2
            xn_t = xn_d.at[slot]

            def perm_kv(b, r0, n, dep):
                masks = _field_masks((n // 2, 128))
                for part, dst in (((1, kf_s), (2, vf_s)) if kvord == 0 else ((2, vf_s), (1, kf_s))):
                    ri = raw_s[pl.ds(pl.multiple_of((b + r0) // 2, 8), n // 2), part * D:(part + 1) * D]
                    cols = [ri[:, c * 128:(c + 1) * 128] for c in range(8)]
                    if dep is not None:
                        dz = dep if n == UNIT else jnp.concatenate([dep] * (n // UNIT), axis=0)
                        cols = [c | dz for c in cols]
                    cols = _permute(cols, masks)
                    for j in range(8):
                        dst[j, r0:r0 + n, :] = pltpu.bitcast(cols[j], bf16).astype(f32)

            def attn(b, lb, dep):
                R = UNIT
                row = jax.lax.broadcasted_iota(i32, (R, 128), 0) + (t * TM + b)
                lane = jax.lax.broadcasted_iota(i32, (R, 128), 1)
                odd = (lane & 1) == 1
                hi16 = (lane & 16) != 0
                masks = _field_masks((R // 2, 128))
                qi = raw_s[pl.ds(pl.multiple_of((b + HALO) // 2, 8), R // 2), 0:D]
                qc = _permute([qi[:, c * 128:(c + 1) * 128] for c in range(8)], masks)
                if dep is not None and qdep == 0:
                    qc = [c | dep for c in qc]
                if dep is not None and qdep == 2:
                    qc = [c | dep if i < 4 else c for i, c in enumerate(qc)]
                q = [pltpu.bitcast(c, bf16).astype(f32) * c_scale for c in qc]
                if dep is not None and qdep == 1:
                    dd = pltpu.bitcast(jnp.concatenate([dep, dep], axis=0), f32)
                    q = [c + dd for c in q]
                z = []
                for w in range(WIN):
                    st = pl.ds(lb + HALO - DIL * w, R)
                    zw = q[0] * kf_s[0, st, :]
                    for j in range(1, 8):
                        zw = zw + q[j] * kf_s[j, st, :]
                    zw = zw + jnp.where(odd, pltpu.roll(zw, 1, 1), pltpu.roll(zw, 127, 1))
                    zw = zw + jnp.where(hi16, pltpu.roll(zw, 16, 1), pltpu.roll(zw, 112, 1))
                    if w > 0:
                        zw = jnp.where(row >= DIL * w, zw, -1e9)
                    z.append(zw)
                mx = z[0]
                for w in range(1, WIN):
                    mx = jnp.maximum(mx, z[w])
                e = [jnp.exp2(zw - mx) for zw in z]
                den = e[0]
                for w in range(1, WIN):
                    den = den + e[w]
                rden = 1.0 / den
                a = [ew * rden for ew in e]
                outs = []
                for j in range(8):
                    o = a[0] * vf_s[j, pl.ds(lb + HALO, R), :]
                    for w in range(1, WIN):
                        o = o + a[w] * vf_s[j, pl.ds(lb + HALO - DIL * w, R), :]
                    outs.append(pltpu.bitcast(o.astype(bf16), i32))
                nat = _permute(outs, masks)
                for c in range(8):
                    ob_s[pl.ds(pl.multiple_of(b // 2, 8), R // 2), c * 128:(c + 1) * 128] = nat[c]
                return pltpu.bitcast({'rden': rden, 'mx': mx, 'den': den, 'a7': a[7], 'a0': a[0], 'z7': z[7]}[link], i32)[tok * 8:tok * 8 + 8, :]

            def trip(f, c):
                @pl.when(t == 0)
                def _():
                    for cp in tcopies(f): cp.wait()
                with sc('itbody'):
                    for k in range(SUB):
                        ffn(xn_t, pl.multiple_of(FC0 + f * FT + k * FC, 128), FC, False)
                    b0 = [pl.multiple_of(f * RPT, RPT), pl.multiple_of(f * RPT, 16), pl.multiple_of(jnp.minimum(f * RPT, TM - RPT), 16)][bv]
                    zero = jnp.full((UNIT // 2, 128), [jnp.minimum(f, 0), f >> 8, jnp.minimum(t, 0)][zv], i32)
                    dep = None
                    zero2 = jnp.full((UNIT // 2, 128), f >> 8, i32)
                    for u in range(RPT // UNIT):
                        bu = pl.multiple_of(b0 + u * UNIT, UNIT)
                        if u == 0:
                            perm_kv(b0, 0, HALO + UNIT, None)
                        else:
                            perm_kv(b0, HALO + u * UNIT, UNIT, dep)
                        def ln(dp):
                            rs = pl.ds(bu, UNIT)
                            if dp is None:
                                xn_d[1 - slot, rs, :] = _layernorm(xb_d[1 - slot, rs, :])
                            else:
                                xi = xb[1 - slot, pl.ds(pl.multiple_of(bu // 2, 8), UNIT // 2), :] | jnp.concatenate([dp] * 8, axis=1)
                                xn_d[1 - slot, rs, :] = _layernorm(pltpu.bitcast(xi, bf16))
                        prev = dep
                        if var in (3, 4): ln(prev if var == 3 else None)
                        raw = attn(bu, u * UNIT, dep)
                        dep = raw & zero
                        if andin: dep_ln = raw & zero2
                        else: dep_ln = dep
                        if var == 0: ln(dep_ln)
                        elif var == 1: ln(None)
                        elif var == 2: ln(prev)
                return c

            with sc('twait'):
                @pl.when(t + 1 < NT)
                def _():
                    xcopy(t + 1).wait()
            jax.lax.fori_loop(0, NTRIP, trip, 0)

            with sc('wowait'):
                @pl.when(t == 0)
                def _():
                    wocopy().wait()

                @pl.when(t >= 2)
                def _():
                    for r in range(len(OBS)): ocopy(t - 2, r).wait()
            with sc('wo'):
                raw_s[0:HALO // 2, D:3 * D] = raw_s[TM // 2:(TM + HALO) // 2, D:3 * D]
                ss = [jnp.dot(ob_d[OST[r]:OST[r] + OBS[r], :], wo_d[...], preferred_element_type=f32)
                      for r in range(len(OBS))]
                for r in range(len(OBS)):
                    rs = slice(OST[r], OST[r] + OBS[r])
                    out_d[slot, rs, :] = (xb_d[slot, rs, :].astype(f32) + ss[r] * _silu(acc_s[rs, :])).astype(bf16)
                    ocopy(t, r).start()

                @pl.when(t + 2 < NT)
                def _():
                    xcopy(t + 2).start()
            with sc('front'):
                @pl.when(t + 1 < NT)
                def _():
                    xn_n = xn_d.at[1 - slot]
                    ffn(xn_n, 0, FC0, True)
                    for part in range(3):
                        cs = slice(part * D, (part + 1) * D)
                        r = jnp.dot(xn_n[...], wqkv_d[:, cs], preferred_element_type=f32)
                        raw_d[HALO:HALO + TM, cs] = r.astype(bf16)
            return carry

        def tile_s(t, c):
            with sc('tile'):
                return tile(t, c)
        jax.lax.fori_loop(0, NT, tile_s, 0)
        for t in range(NT - 2, NT):
            for r in range(len(OBS)): ocopy(t, r).wait()

    anyspec = pl.BlockSpec(memory_space=pl.ANY)

    @jax.jit
    def fn(x, wqkv, wo, bx, w1, w3, w2):
        out = pl.pallas_call(
            kern,
            in_specs=[anyspec] * 6,
            out_specs=anyspec,
            out_shape=jax.ShapeDtypeStruct((S, D), bf16),
            scratch_shapes=[
                pltpu.VMEM((2, TM // 2, D), i32), pltpu.VMEM((D // 2, 3 * D), i32), pltpu.VMEM((D // 2, D), i32),
                pltpu.VMEM((D // 2, F), i32), pltpu.VMEM((D // 2, F), i32), pltpu.VMEM((F // 2, D), i32),
                pltpu.VMEM((2, TM // 2, D), i32), pltpu.VMEM((2, TM // 2, D), i32),
                pltpu.VMEM(((TM + HALO) // 2, 3 * D), i32),
                pltpu.VMEM((8, RPT + HALO, 128), f32), pltpu.VMEM((8, RPT + HALO, 128), f32),
                pltpu.VMEM((TM // 2, D), i32), pltpu.VMEM((TM, D), f32),
                pltpu.SemaphoreType.DMA((XP,)), pltpu.SemaphoreType.DMA((2,)), pltpu.SemaphoreType.DMA((2, len(OBS))),
                pltpu.SemaphoreType.DMA((3, NP)), pltpu.SemaphoreType.DMA((NQ,)), pltpu.SemaphoreType.DMA((3, NTRIP + 1))],
            compiler_params=pltpu.CompilerParams(vmem_limit_bytes=110 * 2**20),
        )(x[0], wqkv, wo, w1, w3, w2)
        return out[None]
    return fn


_fn = mk(**dict(tok=1))


@jax.jit
def pallas_recurrent_scan__sliding_local_dilated__glu_gated_swiglu__prompt_kernel(
    A_x, A_wqkv, A_wo, B_x, B_w1, B_w3, B_w2
):
    return _fn(A_x, A_wqkv, A_wo, B_x, B_w1, B_w3, B_w2)
```

```python
import contextlib
import jax
import jax.numpy as jnp
import numpy as np
from jax.experimental import pallas as pl
from jax.experimental.pallas import tpu as pltpu

S, D, F = 2048, 1024, 3584
f32, bf16, i32 = jnp.float32, jnp.bfloat16, jnp.int32
HALO = 16
WIN, DIL = 8, 2


def _field_masks(shape):
    lane = jax.lax.broadcasted_iota(i32, shape, len(shape) - 1)
    fld = (lane >> 1) & 7
    return [((fld >> b) & 1) == 1 for b in range(3)]


def _permute(cols, masks):
    r = [cols[c] if c == 0 else pltpu.roll(cols[c], 2 * c, 1) for c in range(8)]
    x = [r[(-c) % 8] for c in range(8)]
    for b in range(3):
        x = [jnp.where(masks[b], x[(j - (1 << b)) % 8], x[j]) for j in range(8)]
    return [x[j] if j == 0 else pltpu.roll(x[j], 128 - 2 * j, 1) for j in range(8)]


def _silu(g):
    hg = 0.5 * g
    return hg + hg * jnp.tanh(hg)


def _layernorm(x):
    x = x.astype(f32)
    m = jnp.mean(x, axis=-1, keepdims=True)
    xc = x - m
    var = jnp.mean(xc * xc, axis=-1, keepdims=True)
    return (xc * jax.lax.rsqrt(var + 1e-5)).astype(bf16)


def mk(TM=512, FC0=512, NTRIP=4, SUB=2, PF=128, PQ=768, OBS=(384, 128), LNR=128, link='rden', early=1, prof=False,
       trip_wait=1, XP=2, var=0, bv=0, zv=0, tok=0, andin=0, slotv=0, kvord=0, qdep=0, flags=None, nochain=0):
    UNIT = 16
    FT = (F - FC0) // NTRIP
    FC = FT // SUB
    RPT = TM // NTRIP
    NT = S // TM
    NP, NQ = FC0 // PF, 3 * D // PQ
    OST = [sum(OBS[:r]) for r in range(len(OBS))]
    XR = TM // XP
    assert FC0 + NTRIP * SUB * FC == F and FC % 128 == 0 and RPT % UNIT == 0 and sum(OBS) == TM
    c_scale = float((D // 32) ** 0 * 32 ** -0.5 * np.log2(np.e))
    sc = lambda n: (jax.named_scope(n) if (prof is True or (prof and (n in prof or n.startswith('pro'))))
                    else contextlib.nullcontext())

    def kern(x_hbm, wqkv_hbm, wo_hbm, w1_hbm, w3_hbm, w2_hbm, o_hbm,
             xb, wqkv_s, wo_s, w1_s, w3_s, w2_s, out_s, xn_s, raw_s, kf_s, vf_s, ob_s, acc_s,
             x0sem, xsem, osem, psem, qsem, tsem):
        xb_d, wqkv_d, wo_d, w1_d, w3_d, w2_d, out_d, xn_d, raw_d, ob_d = [
            r.bitcast(bf16) for r in (xb, wqkv_s, wo_s, w1_s, w3_s, w2_s, out_s, xn_s, raw_s, ob_s)]

        def x0copy(p):
            rs = pl.ds(pl.multiple_of(p * XR, XR), XR)
            return pltpu.make_async_copy(x_hbm.at[rs, :], xb_d.at[0, rs, :], x0sem.at[p])

        def xcopy(t):
            return pltpu.make_async_copy(x_hbm.at[pl.ds(pl.multiple_of(t * TM, TM), TM), :],
                                         xb_d.at[t & 1], xsem.at[t & 1])

        def ocopy(t, r):
            return pltpu.make_async_copy(out_d.at[t & 1, pl.ds(OST[r], OBS[r]), :],
                                         o_hbm.at[pl.ds(pl.multiple_of(t * TM + OST[r], 16), OBS[r]), :],
                                         osem.at[t & 1, r])

        def fcopies(start, n, sems, i):
            sl = pl.ds(start, n)
            return [pltpu.make_async_copy(w1_hbm.at[:, sl], w1_d.at[:, sl], sems.at[0, i]),
                    pltpu.make_async_copy(w3_hbm.at[:, sl], w3_d.at[:, sl], sems.at[1, i]),
                    pltpu.make_async_copy(w2_hbm.at[sl, :], w2_d.at[sl, :], sems.at[2, i])]

        pcopies = lambda i: fcopies(pl.multiple_of(i * PF, PF), PF, psem, i)
        tcopies = lambda f: fcopies(pl.multiple_of(FC0 + f * FT, 128), FT, tsem, f)

        def qcopy(i):
            sl = pl.ds(pl.multiple_of(i * PQ, 128), PQ)
            return pltpu.make_async_copy(wqkv_hbm.at[:, sl], wqkv_d.at[:, sl], qsem.at[i])

        def wocopy():
            return pltpu.make_async_copy(wo_hbm, wo_d, tsem.at[0, NTRIP])

        def ffn(xn, start, n, init):
            sl = pl.ds(start, n)
            g = jnp.dot(xn[...], w1_d[:, sl], preferred_element_type=f32)
            u = jnp.dot(xn[...], w3_d[:, sl], preferred_element_type=f32)
            h = (_silu(g) * u).astype(bf16)
            d = jnp.dot(h, w2_d[sl, :], preferred_element_type=f32)
            if init:
                acc_s[...] = d
            else:
                acc_s[...] += d

        def late_starts(k):
            if k == 0:
                xcopy(1).start()
                for c in tcopies(0) + tcopies(1): c.start()
            elif k == 1:
                for f in range(2, NTRIP):
                    for c in tcopies(f): c.start()
                wocopy().start()

        with sc('pro_issue'):
            for p in range(XP): x0copy(p).start()
            for i in range(NP):
                for c in pcopies(i): c.start()
            for i in range(NQ): qcopy(i).start()
            for k in range(early): late_starts(k)
            raw_s[0:HALO // 2, D:3 * D] = jnp.zeros((HALO // 2, 2 * D), i32)

            def zero_acc(i, c):
                acc_s[pl.ds(pl.multiple_of(i * 64, 64), 64), :] = jnp.zeros((64, D), f32)
                return c
            jax.lax.fori_loop(0, TM // 64, zero_acc, 0)

        def pro_ln(p, c):
            with sc('pro_xwait'):
                x0copy(p).wait()
            with sc('pro_ln'):
                def rows(i, c2):
                    rs = pl.ds(pl.multiple_of(p * XR + i * LNR, LNR), LNR)
                    xn_d[0, rs, :] = _layernorm(xb_d[0, rs, :])
                    return c2
                jax.lax.fori_loop(0, XR // LNR, rows, 0)
            return c
        jax.lax.fori_loop(0, XP, pro_ln, 0)

        def pro_ffn(i, c):
            for cp in pcopies(i): cp.wait()
            with sc('pro_ffn'):
                ffn(xn_d.at[0], pl.multiple_of(i * PF, PF), PF, False)
            return c
        jax.lax.fori_loop(0, NP, pro_ffn, 0)
        for k in range(early, 2): late_starts(k)

        def pro_qkv(i, c):
            qcopy(i).wait()
            with sc('pro_qkv'):
                cs = pl.ds(pl.multiple_of(i * PQ, 128), PQ)
                r = jnp.dot(xn_d[0], wqkv_d[:, cs], preferred_element_type=f32)
                raw_d[HALO:HALO + TM, cs] = r.astype(bf16)
            return c
        jax.lax.fori_loop(0, NQ, pro_qkv, 0)

        def tile(t, carry):
            slot = (t & 1) if slotv == 0 else t % 2
            xn_t = xn_d.at[slot]

            def perm_kv(b, r0, n, dep):
                masks = _field_masks((n // 2, 128))
                for part, dst in (((1, kf_s), (2, vf_s)) if kvord == 0 else ((2, vf_s), (1, kf_s))):
                    ri = raw_s[pl.ds(pl.multiple_of((b + r0) // 2, 8), n // 2), part * D:(part + 1) * D]
                    cols = [ri[:, c * 128:(c + 1) * 128] for c in range(8)]
                    if dep is not None:
                        dz = dep if n == UNIT else jnp.concatenate([dep] * (n // UNIT), axis=0)
                        cols = [c | dz for c in cols]
                    cols = _permute(cols, masks)
                    for j in range(8):
                        dst[j, r0:r0 + n, :] = pltpu.bitcast(cols[j], bf16).astype(f32)

            def attn(b, lb, dep):
                R = UNIT
                row = jax.lax.broadcasted_iota(i32, (R, 128), 0) + (t * TM + b)
                lane = jax.lax.broadcasted_iota(i32, (R, 128), 1)
                odd = (lane & 1) == 1
                hi16 = (lane & 16) != 0
                masks = _field_masks((R // 2, 128))
                qi = raw_s[pl.ds(pl.multiple_of((b + HALO) // 2, 8), R // 2), 0:D]
                qc = _permute([qi[:, c * 128:(c + 1) * 128] for c in range(8)], masks)
                if dep is not None and qdep == 0:
                    qc = [c | dep for c in qc]
                if dep is not None and qdep == 2:
                    qc = [c | dep if i < 4 else c for i, c in enumerate(qc)]
                q = [pltpu.bitcast(c, bf16).astype(f32) * c_scale for c in qc]
                if dep is not None and qdep == 1:
                    dd = pltpu.bitcast(jnp.concatenate([dep, dep], axis=0), f32)
                    q = [c + dd for c in q]
                z = []
                for w in range(WIN):
                    st = pl.ds(lb + HALO - DIL * w, R)
                    zw = q[0] * kf_s[0, st, :]
                    for j in range(1, 8):
                        zw = zw + q[j] * kf_s[j, st, :]
                    zw = zw + jnp.where(odd, pltpu.roll(zw, 1, 1), pltpu.roll(zw, 127, 1))
                    zw = zw + jnp.where(hi16, pltpu.roll(zw, 16, 1), pltpu.roll(zw, 112, 1))
                    if w > 0:
                        zw = jnp.where(row >= DIL * w, zw, -1e9)
                    z.append(zw)
                mx = z[0]
                for w in range(1, WIN):
                    mx = jnp.maximum(mx, z[w])
                e = [jnp.exp2(zw - mx) for zw in z]
                den = e[0]
                for w in range(1, WIN):
                    den = den + e[w]
                rden = 1.0 / den
                a = [ew * rden for ew in e]
                outs = []
                for j in range(8):
                    o = a[0] * vf_s[j, pl.ds(lb + HALO, R), :]
                    for w in range(1, WIN):
                        o = o + a[w] * vf_s[j, pl.ds(lb + HALO - DIL * w, R), :]
                    outs.append(pltpu.bitcast(o.astype(bf16), i32))
                nat = _permute(outs, masks)
                for c in range(8):
                    ob_s[pl.ds(pl.multiple_of(b // 2, 8), R // 2), c * 128:(c + 1) * 128] = nat[c]
                return pltpu.bitcast({'rden': rden, 'mx': mx, 'den': den, 'a7': a[7], 'a0': a[0], 'z7': z[7]}[link], i32)[tok * 8:tok * 8 + 8, :]

            def trip(f, c):
                @pl.when(t == 0)
                def _():
                    for cp in tcopies(f): cp.wait()
                with sc('itbody'):
                    for k in range(SUB):
                        ffn(xn_t, pl.multiple_of(FC0 + f * FT + k * FC, 128), FC, False)
                    b0 = [pl.multiple_of(f * RPT, RPT), pl.multiple_of(f * RPT, 16), pl.multiple_of(jnp.minimum(f * RPT, TM - RPT), 16)][bv]
                    zero = jnp.full((UNIT // 2, 128), [jnp.minimum(f, 0), f >> 8, jnp.minimum(t, 0)][zv], i32)
                    dep = None
                    zero2 = jnp.full((UNIT // 2, 128), f >> 8, i32)
                    for u in range(RPT // UNIT):
                        bu = pl.multiple_of(b0 + u * UNIT, UNIT)
                        if u == 0:
                            perm_kv(b0, 0, HALO + UNIT, None)
                        else:
                            perm_kv(b0, HALO + u * UNIT, UNIT, dep)
                        def ln(dp):
                            rs = pl.ds(bu, UNIT)
                            if dp is None:
                                xn_d[1 - slot, rs, :] = _layernorm(xb_d[1 - slot, rs, :])
                            else:
                                xi = xb[1 - slot, pl.ds(pl.multiple_of(bu // 2, 8), UNIT // 2), :] | jnp.concatenate([dp] * 8, axis=1)
                                xn_d[1 - slot, rs, :] = _layernorm(pltpu.bitcast(xi, bf16))
                        prev = dep
                        if var in (3, 4): ln(prev if var == 3 else None)
                        raw = attn(bu, u * UNIT, dep)
                        dep = raw & zero
                        if nochain:
                            if var == 0: ln(None)
                            dep = None
                            continue
                        if andin: dep_ln = raw & zero2
                        else: dep_ln = dep
                        if var == 0: ln(dep_ln)
                        elif var == 1: ln(None)
                        elif var == 2: ln(prev)
                return c

            with sc('twait'):
                @pl.when(t + 1 < NT)
                def _():
                    xcopy(t + 1).wait()
            jax.lax.fori_loop(0, NTRIP, trip, 0)

            with sc('wowait'):
                @pl.when(t == 0)
                def _():
                    wocopy().wait()

                @pl.when(t >= 2)
                def _():
                    for r in range(len(OBS)): ocopy(t - 2, r).wait()
            with sc('wo'):
                raw_s[0:HALO // 2, D:3 * D] = raw_s[TM // 2:(TM + HALO) // 2, D:3 * D]
                ss = [jnp.dot(ob_d[OST[r]:OST[r] + OBS[r], :], wo_d[...], preferred_element_type=f32)
                      for r in range(len(OBS))]
                for r in range(len(OBS)):
                    rs = slice(OST[r], OST[r] + OBS[r])
                    out_d[slot, rs, :] = (xb_d[slot, rs, :].astype(f32) + ss[r] * _silu(acc_s[rs, :])).astype(bf16)
                    ocopy(t, r).start()

                @pl.when(t + 2 < NT)
                def _():
                    xcopy(t + 2).start()
            with sc('front'):
                @pl.when(t + 1 < NT)
                def _():
                    xn_n = xn_d.at[1 - slot]
                    ffn(xn_n, 0, FC0, True)
                    for part in range(3):
                        cs = slice(part * D, (part + 1) * D)
                        r = jnp.dot(xn_n[...], wqkv_d[:, cs], preferred_element_type=f32)
                        raw_d[HALO:HALO + TM, cs] = r.astype(bf16)
            return carry

        def tile_s(t, c):
            with sc('tile'):
                return tile(t, c)
        jax.lax.fori_loop(0, NT, tile_s, 0)
        for t in range(NT - 2, NT):
            for r in range(len(OBS)): ocopy(t, r).wait()

    anyspec = pl.BlockSpec(memory_space=pl.ANY)

    @jax.jit
    def fn(x, wqkv, wo, bx, w1, w3, w2):
        out = pl.pallas_call(
            kern,
            in_specs=[anyspec] * 6,
            out_specs=anyspec,
            out_shape=jax.ShapeDtypeStruct((S, D), bf16),
            scratch_shapes=[
                pltpu.VMEM((2, TM // 2, D), i32), pltpu.VMEM((D // 2, 3 * D), i32), pltpu.VMEM((D // 2, D), i32),
                pltpu.VMEM((D // 2, F), i32), pltpu.VMEM((D // 2, F), i32), pltpu.VMEM((F // 2, D), i32),
                pltpu.VMEM((2, TM // 2, D), i32), pltpu.VMEM((2, TM // 2, D), i32),
                pltpu.VMEM(((TM + HALO) // 2, 3 * D), i32),
                pltpu.VMEM((8, RPT + HALO, 128), f32), pltpu.VMEM((8, RPT + HALO, 128), f32),
                pltpu.VMEM((TM // 2, D), i32), pltpu.VMEM((TM, D), f32),
                pltpu.SemaphoreType.DMA((XP,)), pltpu.SemaphoreType.DMA((2,)), pltpu.SemaphoreType.DMA((2, len(OBS))),
                pltpu.SemaphoreType.DMA((3, NP)), pltpu.SemaphoreType.DMA((NQ,)), pltpu.SemaphoreType.DMA((3, NTRIP + 1))],
            compiler_params=pltpu.CompilerParams(vmem_limit_bytes=110 * 2**20, flags=flags),
        )(x[0], wqkv, wo, w1, w3, w2)
        return out[None]
    return fn


_fn = mk(**dict(link='a0',PQ=1024,OBS=(256,192,64),flags={'XLA_TPU_EVENLY_DISTRIBUTE_CRITICAL_NODES':True}))


@jax.jit
def pallas_recurrent_scan__sliding_local_dilated__glu_gated_swiglu__prompt_kernel(
    A_x, A_wqkv, A_wo, B_x, B_w1, B_w3, B_w2
):
    return _fn(A_x, A_wqkv, A_wo, B_x, B_w1, B_w3, B_w2)
```

```python
import jax
import jax.numpy as jnp
import numpy as np
from jax.experimental import pallas as pl
from jax.experimental.pallas import tpu as pltpu

S, D, F = 2048, 1024, 3584
HEAD_DIM, WIN, DIL = 32, 8, 2
f32, bf16, i32 = jnp.float32, jnp.bfloat16, jnp.int32

TM = 512
NT = S // TM
HALO = 16
FC0 = 512
NTRIP, SUB = 4, 2
FT = (F - FC0) // NTRIP
FC = FT // SUB
RPT = TM // NTRIP
UNIT = 16
PF, PQ = 128, 1024
NP, NQ = FC0 // PF, 3 * D // PQ
XP, LNR = 2, 128
XR = TM // XP
OBS = (256, 192, 64)
OST = (0, 256, 448)
Q_SCALE = float(HEAD_DIM ** -0.5 * np.log2(np.e))


def _field_masks(shape):
    lane = jax.lax.broadcasted_iota(i32, shape, len(shape) - 1)
    fld = (lane >> 1) & 7
    return [((fld >> b) & 1) == 1 for b in range(3)]


def _permute(cols, masks):
    r = [cols[c] if c == 0 else pltpu.roll(cols[c], 2 * c, 1) for c in range(8)]
    x = [r[(-c) % 8] for c in range(8)]
    for b in range(3):
        x = [jnp.where(masks[b], x[(j - (1 << b)) % 8], x[j]) for j in range(8)]
    return [x[j] if j == 0 else pltpu.roll(x[j], 128 - 2 * j, 1) for j in range(8)]


def _silu(g):
    hg = 0.5 * g
    return hg + hg * jnp.tanh(hg)


def _layernorm(x):
    x = x.astype(f32)
    m = jnp.mean(x, axis=-1, keepdims=True)
    xc = x - m
    var = jnp.mean(xc * xc, axis=-1, keepdims=True)
    return (xc * jax.lax.rsqrt(var + 1e-5)).astype(bf16)


def _kernel(x_hbm, wqkv_hbm, wo_hbm, w1_hbm, w3_hbm, w2_hbm, o_hbm,
            xb, wqkv_s, wo_s, w1_s, w3_s, w2_s, out_s, xn_s, raw_s, kf_s, vf_s, ob_s, acc_s,
            x0sem, xsem, osem, psem, qsem, tsem):
    xb_d, wqkv_d, wo_d, w1_d, w3_d, w2_d, out_d, xn_d, raw_d, ob_d = [
        r.bitcast(bf16) for r in (xb, wqkv_s, wo_s, w1_s, w3_s, w2_s, out_s, xn_s, raw_s, ob_s)]

    def x0copy(p):
        rs = pl.ds(pl.multiple_of(p * XR, XR), XR)
        return pltpu.make_async_copy(x_hbm.at[rs, :], xb_d.at[0, rs, :], x0sem.at[p])

    def xcopy(t):
        return pltpu.make_async_copy(x_hbm.at[pl.ds(pl.multiple_of(t * TM, TM), TM), :],
                                     xb_d.at[t & 1], xsem.at[t & 1])

    def ocopy(t, r):
        return pltpu.make_async_copy(out_d.at[t & 1, pl.ds(OST[r], OBS[r]), :],
                                     o_hbm.at[pl.ds(pl.multiple_of(t * TM + OST[r], 16), OBS[r]), :],
                                     osem.at[t & 1, r])

    def fcopies(start, n, sems, i):
        sl = pl.ds(start, n)
        return [pltpu.make_async_copy(w1_hbm.at[:, sl], w1_d.at[:, sl], sems.at[0, i]),
                pltpu.make_async_copy(w3_hbm.at[:, sl], w3_d.at[:, sl], sems.at[1, i]),
                pltpu.make_async_copy(w2_hbm.at[sl, :], w2_d.at[sl, :], sems.at[2, i])]

    def pcopies(i):
        return fcopies(pl.multiple_of(i * PF, PF), PF, psem, i)

    def tcopies(f):
        return fcopies(pl.multiple_of(FC0 + f * FT, 128), FT, tsem, f)

    def qcopy(i):
        sl = pl.ds(pl.multiple_of(i * PQ, 128), PQ)
        return pltpu.make_async_copy(wqkv_hbm.at[:, sl], wqkv_d.at[:, sl], qsem.at[i])

    def wocopy():
        return pltpu.make_async_copy(wo_hbm, wo_d, tsem.at[0, NTRIP])

    def ffn(xn, start, n, init):
        sl = pl.ds(start, n)
        g = jnp.dot(xn[...], w1_d[:, sl], preferred_element_type=f32)
        u = jnp.dot(xn[...], w3_d[:, sl], preferred_element_type=f32)
        h = (_silu(g) * u).astype(bf16)
        d = jnp.dot(h, w2_d[sl, :], preferred_element_type=f32)
        if init:
            acc_s[...] = d
        else:
            acc_s[...] += d

    for p in range(XP):
        x0copy(p).start()
    for i in range(NP):
        for c in pcopies(i):
            c.start()
    for i in range(NQ):
        qcopy(i).start()
    xcopy(1).start()
    for c in tcopies(0) + tcopies(1):
        c.start()
    raw_s[0:HALO // 2, D:3 * D] = jnp.zeros((HALO // 2, 2 * D), i32)

    def zero_acc(i, c):
        acc_s[pl.ds(pl.multiple_of(i * 64, 64), 64), :] = jnp.zeros((64, D), f32)
        return c
    jax.lax.fori_loop(0, TM // 64, zero_acc, 0)

    def pro_ln(p, c):
        x0copy(p).wait()

        def rows(i, c2):
            rs = pl.ds(pl.multiple_of(p * XR + i * LNR, LNR), LNR)
            xn_d[0, rs, :] = _layernorm(xb_d[0, rs, :])
            return c2
        jax.lax.fori_loop(0, XR // LNR, rows, 0)
        return c
    jax.lax.fori_loop(0, XP, pro_ln, 0)

    def pro_ffn(i, c):
        for cp in pcopies(i):
            cp.wait()
        ffn(xn_d.at[0], pl.multiple_of(i * PF, PF), PF, False)
        return c
    jax.lax.fori_loop(0, NP, pro_ffn, 0)
    for f in range(2, NTRIP):
        for c in tcopies(f):
            c.start()
    wocopy().start()

    def pro_qkv(i, c):
        qcopy(i).wait()
        cs = pl.ds(pl.multiple_of(i * PQ, 128), PQ)
        r = jnp.dot(xn_d[0], wqkv_d[:, cs], preferred_element_type=f32)
        raw_d[HALO:HALO + TM, cs] = r.astype(bf16)
        return c
    jax.lax.fori_loop(0, NQ, pro_qkv, 0)

    def tile(t, carry):
        slot = t & 1
        xn_t = xn_d.at[slot]

        def perm_kv(b, r0, n, dep):
            masks = _field_masks((n // 2, 128))
            for part, dst in ((1, kf_s), (2, vf_s)):
                ri = raw_s[pl.ds(pl.multiple_of((b + r0) // 2, 8), n // 2), part * D:(part + 1) * D]
                cols = [ri[:, c * 128:(c + 1) * 128] for c in range(8)]
                if dep is not None:
                    cols = [c | dep for c in cols]
                cols = _permute(cols, masks)
                for j in range(8):
                    dst[j, r0:r0 + n, :] = pltpu.bitcast(cols[j], bf16).astype(f32)

        def attn(b, lb, dep):
            R = UNIT
            row = jax.lax.broadcasted_iota(i32, (R, 128), 0) + (t * TM + b)
            lane = jax.lax.broadcasted_iota(i32, (R, 128), 1)
            odd = (lane & 1) == 1
            hi16 = (lane & 16) != 0
            masks = _field_masks((R // 2, 128))
            qi = raw_s[pl.ds(pl.multiple_of((b + HALO) // 2, 8), R // 2), 0:D]
            qc = _permute([qi[:, c * 128:(c + 1) * 128] for c in range(8)], masks)
            if dep is not None:
                qc = [c | dep for c in qc]
            q = [pltpu.bitcast(c, bf16).astype(f32) * Q_SCALE for c in qc]
            z = []
            for w in range(WIN):
                st = pl.ds(lb + HALO - DIL * w, R)
                zw = q[0] * kf_s[0, st, :]
                for j in range(1, 8):
                    zw = zw + q[j] * kf_s[j, st, :]
                zw = zw + jnp.where(odd, pltpu.roll(zw, 1, 1), pltpu.roll(zw, 127, 1))
                zw = zw + jnp.where(hi16, pltpu.roll(zw, 16, 1), pltpu.roll(zw, 112, 1))
                if w > 0:
                    zw = jnp.where(row >= DIL * w, zw, -1e9)
                z.append(zw)
            mx = z[0]
            for w in range(1, WIN):
                mx = jnp.maximum(mx, z[w])
            e = [jnp.exp2(zw - mx) for zw in z]
            den = e[0]
            for w in range(1, WIN):
                den = den + e[w]
            rden = 1.0 / den
            a = [ew * rden for ew in e]
            outs = []
            for j in range(8):
                o = a[0] * vf_s[j, pl.ds(lb + HALO, R), :]
                for w in range(1, WIN):
                    o = o + a[w] * vf_s[j, pl.ds(lb + HALO - DIL * w, R), :]
                outs.append(pltpu.bitcast(o.astype(bf16), i32))
            nat = _permute(outs, masks)
            for c in range(8):
                ob_s[pl.ds(pl.multiple_of(b // 2, 8), R // 2), c * 128:(c + 1) * 128] = nat[c]
            return pltpu.bitcast(a[0], i32)[0:R // 2, :]

        def trip(f, c):
            @pl.when(t == 0)
            def _():
                for cp in tcopies(f):
                    cp.wait()
            for k in range(SUB):
                ffn(xn_t, pl.multiple_of(FC0 + f * FT + k * FC, 128), FC, False)
            b0 = pl.multiple_of(f * RPT, RPT)
            zero = jnp.full((UNIT // 2, 128), jnp.minimum(f, 0), i32)
            dep = None
            for u in range(RPT // UNIT):
                bu = pl.multiple_of(b0 + u * UNIT, UNIT)
                if u == 0:
                    perm_kv(b0, 0, HALO + UNIT, None)
                else:
                    perm_kv(b0, HALO + u * UNIT, UNIT, dep)
                dep = attn(bu, u * UNIT, dep) & zero
                xi = xb[1 - slot, pl.ds(pl.multiple_of(bu // 2, 8), UNIT // 2), :]
                xi = xi | jnp.concatenate([dep] * 8, axis=1)
                xn_d[1 - slot, pl.ds(bu, UNIT), :] = _layernorm(pltpu.bitcast(xi, bf16))
            return c

        @pl.when(t + 1 < NT)
        def _():
            xcopy(t + 1).wait()
        jax.lax.fori_loop(0, NTRIP, trip, 0)

        @pl.when(t == 0)
        def _():
            wocopy().wait()

        @pl.when(t >= 2)
        def _():
            for r in range(len(OBS)):
                ocopy(t - 2, r).wait()

        raw_s[0:HALO // 2, D:3 * D] = raw_s[TM // 2:(TM + HALO) // 2, D:3 * D]
        ss = [jnp.dot(ob_d[OST[r]:OST[r] + OBS[r], :], wo_d[...], preferred_element_type=f32)
              for r in range(len(OBS))]
        for r in range(len(OBS)):
            rs = slice(OST[r], OST[r] + OBS[r])
            out_d[slot, rs, :] = (xb_d[slot, rs, :].astype(f32) + ss[r] * _silu(acc_s[rs, :])).astype(bf16)
            ocopy(t, r).start()

        @pl.when(t + 2 < NT)
        def _():
            xcopy(t + 2).start()

        @pl.when(t + 1 < NT)
        def _():
            xn_n = xn_d.at[1 - slot]
            ffn(xn_n, 0, FC0, True)
            for part in range(3):
                cs = slice(part * D, (part + 1) * D)
                r = jnp.dot(xn_n[...], wqkv_d[:, cs], preferred_element_type=f32)
                raw_d[HALO:HALO + TM, cs] = r.astype(bf16)
        return carry

    jax.lax.fori_loop(0, NT, tile, 0)
    for t in range(NT - 2, NT):
        for r in range(len(OBS)):
            ocopy(t, r).wait()


@jax.jit
def pallas_recurrent_scan__sliding_local_dilated__glu_gated_swiglu__prompt_kernel(
    A_x: jax.Array,
    A_wqkv: jax.Array,
    A_wo: jax.Array,
    B_x: jax.Array,
    B_w1: jax.Array,
    B_w3: jax.Array,
    B_w2: jax.Array,
):
    del B_x
    anyspec = pl.BlockSpec(memory_space=pl.ANY)
    out = pl.pallas_call(
        _kernel,
        in_specs=[anyspec] * 6,
        out_specs=anyspec,
        out_shape=jax.ShapeDtypeStruct((S, D), bf16),
        scratch_shapes=[
            pltpu.VMEM((2, TM // 2, D), i32),
            pltpu.VMEM((D // 2, 3 * D), i32),
            pltpu.VMEM((D // 2, D), i32),
            pltpu.VMEM((D // 2, F), i32),
            pltpu.VMEM((D // 2, F), i32),
            pltpu.VMEM((F // 2, D), i32),
            pltpu.VMEM((2, TM // 2, D), i32),
            pltpu.VMEM((2, TM // 2, D), i32),
            pltpu.VMEM(((TM + HALO) // 2, 3 * D), i32),
            pltpu.VMEM((8, RPT + HALO, 128), f32),
            pltpu.VMEM((8, RPT + HALO, 128), f32),
            pltpu.VMEM((TM // 2, D), i32),
            pltpu.VMEM((TM, D), f32),
            pltpu.SemaphoreType.DMA((XP,)),
            pltpu.SemaphoreType.DMA((2,)),
            pltpu.SemaphoreType.DMA((2, len(OBS))),
            pltpu.SemaphoreType.DMA((3, NP)),
            pltpu.SemaphoreType.DMA((NQ,)),
            pltpu.SemaphoreType.DMA((3, NTRIP + 1)),
        ],
        compiler_params=pltpu.CompilerParams(
            vmem_limit_bytes=110 * 2**20,
            flags={"XLA_TPU_EVENLY_DISTRIBUTE_CRITICAL_NODES": True},
        ),
    )(A_x[0], A_wqkv, A_wo, B_w1, B_w3, B_w2)
    return out[None]
```

```python
import jax
import jax.numpy as jnp
import numpy as np
from jax.experimental import pallas as pl
from jax.experimental.pallas import tpu as pltpu

S, D, F = 2048, 1024, 3584
HEAD_DIM, WIN, DIL = 32, 8, 2
f32, bf16, i32 = jnp.float32, jnp.bfloat16, jnp.int32

TM = 512
NT = S // TM
HALO = 16
FC0 = 512
NTRIP, SUB = 4, 2
FT = (F - FC0) // NTRIP
FC = FT // SUB
RPT = TM // NTRIP
UNIT = 16
PF, PQ = 128, 1024
NP, NQ = FC0 // PF, 3 * D // PQ
XP, LNR = 2, 128
XR = TM // XP
OBS = (256, 192, 64)
OST = (0, 256, 448)
Q_SCALE = float(HEAD_DIM ** -0.5 * np.log2(np.e))


def _field_masks(shape):
    lane = jax.lax.broadcasted_iota(i32, shape, len(shape) - 1)
    fld = (lane >> 1) & 7
    return [((fld >> b) & 1) == 1 for b in range(3)]


def _permute(cols, masks):
    r = [cols[c] if c == 0 else pltpu.roll(cols[c], 2 * c, 1) for c in range(8)]
    x = [r[(-c) % 8] for c in range(8)]
    for b in range(3):
        x = [jnp.where(masks[b], x[(j - (1 << b)) % 8], x[j]) for j in range(8)]
    return [x[j] if j == 0 else pltpu.roll(x[j], 128 - 2 * j, 1) for j in range(8)]


def _silu(g):
    hg = 0.5 * g
    return hg + hg * jnp.tanh(hg)


def _layernorm(x):
    x = x.astype(f32)
    m = jnp.mean(x, axis=-1, keepdims=True)
    xc = x - m
    var = jnp.mean(xc * xc, axis=-1, keepdims=True)
    return (xc * jax.lax.rsqrt(var + 1e-5)).astype(bf16)


def _kernel(x_hbm, wqkv_hbm, wo_hbm, w1_hbm, w3_hbm, w2_hbm, o_hbm,
            xb, wqkv_s, wo_s, w1_s, w3_s, w2_s, out_s, xn_s, raw_s, kf_s, vf_s, ob_s, acc_s,
            x0sem, xsem, osem, psem, qsem, tsem):
    xb_d, wqkv_d, wo_d, w1_d, w3_d, w2_d, out_d, xn_d, raw_d, ob_d = [
        r.bitcast(bf16) for r in (xb, wqkv_s, wo_s, w1_s, w3_s, w2_s, out_s, xn_s, raw_s, ob_s)]

    def x0copy(p):
        rs = pl.ds(pl.multiple_of(p * XR, XR), XR)
        return pltpu.make_async_copy(x_hbm.at[rs, :], xb_d.at[0, rs, :], x0sem.at[p])

    def xcopy(t):
        return pltpu.make_async_copy(x_hbm.at[pl.ds(pl.multiple_of(t * TM, TM), TM), :],
                                     xb_d.at[t & 1], xsem.at[t & 1])

    def ocopy(t, r):
        return pltpu.make_async_copy(out_d.at[t & 1, pl.ds(OST[r], OBS[r]), :],
                                     o_hbm.at[pl.ds(pl.multiple_of(t * TM + OST[r], 16), OBS[r]), :],
                                     osem.at[t & 1, r])

    def fcopies(start, n, sems, i):
        sl = pl.ds(start, n)
        return [pltpu.make_async_copy(w1_hbm.at[:, sl], w1_d.at[:, sl], sems.at[0, i]),
                pltpu.make_async_copy(w3_hbm.at[:, sl], w3_d.at[:, sl], sems.at[1, i]),
                pltpu.make_async_copy(w2_hbm.at[sl, :], w2_d.at[sl, :], sems.at[2, i])]

    def pcopies(i):
        return fcopies(pl.multiple_of(i * PF, PF), PF, psem, i)

    def tcopies(f):
        return fcopies(pl.multiple_of(FC0 + f * FT, 128), FT, tsem, f)

    def qcopy(i):
        sl = pl.ds(pl.multiple_of(i * PQ, 128), PQ)
        return pltpu.make_async_copy(wqkv_hbm.at[:, sl], wqkv_d.at[:, sl], qsem.at[i])

    def wocopy():
        return pltpu.make_async_copy(wo_hbm, wo_d, tsem.at[0, NTRIP])

    def ffn(xn, start, n, init):
        sl = pl.ds(start, n)
        g = jnp.dot(xn[...], w1_d[:, sl], preferred_element_type=f32)
        u = jnp.dot(xn[...], w3_d[:, sl], preferred_element_type=f32)
        h = (_silu(g) * u).astype(bf16)
        d = jnp.dot(h, w2_d[sl, :], preferred_element_type=f32)
        if init:
            acc_s[...] = d
        else:
            acc_s[...] += d

    for p in range(XP):
        x0copy(p).start()
    for i in range(NP):
        for c in pcopies(i):
            c.start()
    for i in range(NQ):
        qcopy(i).start()
    xcopy(1).start()
    for c in tcopies(0) + tcopies(1):
        c.start()
    raw_d[0:HALO, D:3 * D] = jnp.zeros((HALO, 2 * D), bf16)

    def zero_acc(i, c):
        acc_s[pl.ds(pl.multiple_of(i * 64, 64), 64), :] = jnp.zeros((64, D), f32)
        return c
    jax.lax.fori_loop(0, TM // 64, zero_acc, 0)

    def pro_ln(p, c):
        x0copy(p).wait()

        def rows(i, c2):
            rs = pl.ds(pl.multiple_of(p * XR + i * LNR, LNR), LNR)
            xn_d[0, rs, :] = _layernorm(xb_d[0, rs, :])
            return c2
        jax.lax.fori_loop(0, XR // LNR, rows, 0)
        return c
    jax.lax.fori_loop(0, XP, pro_ln, 0)

    def pro_ffn(i, c):
        for cp in pcopies(i):
            cp.wait()
        ffn(xn_d.at[0], pl.multiple_of(i * PF, PF), PF, False)
        return c
    jax.lax.fori_loop(0, NP, pro_ffn, 0)
    for f in range(2, NTRIP):
        for c in tcopies(f):
            c.start()
    wocopy().start()

    def pro_qkv(i, c):
        qcopy(i).wait()
        cs = pl.ds(pl.multiple_of(i * PQ, 128), PQ)
        r = jnp.dot(xn_d[0], wqkv_d[:, cs], preferred_element_type=f32)
        raw_d[HALO:HALO + TM, cs] = r.astype(bf16)
        return c
    jax.lax.fori_loop(0, NQ, pro_qkv, 0)

    def tile(t, carry):
        slot = t & 1
        xn_t = xn_d.at[slot]

        def perm_kv(b, r0, n, dep):
            masks = _field_masks((n // 2, 128))
            for part, dst in ((1, kf_s), (2, vf_s)):
                ri = pltpu.bitcast(raw_d[pl.ds(pl.multiple_of(b + r0, 16), n), part * D:(part + 1) * D], i32)
                cols = [ri[:, c * 128:(c + 1) * 128] for c in range(8)]
                if dep is not None:
                    cols = [c | dep for c in cols]
                cols = _permute(cols, masks)
                for j in range(8):
                    dst[j, r0:r0 + n, :] = pltpu.bitcast(cols[j], bf16).astype(f32)

        def attn(b, lb, dep):
            R = UNIT
            row = jax.lax.broadcasted_iota(i32, (R, 128), 0) + (t * TM + b)
            lane = jax.lax.broadcasted_iota(i32, (R, 128), 1)
            odd = (lane & 1) == 1
            hi16 = (lane & 16) != 0
            masks = _field_masks((R // 2, 128))
            qi = pltpu.bitcast(raw_d[pl.ds(pl.multiple_of(b + HALO, 16), R), 0:D], i32)
            qc = _permute([qi[:, c * 128:(c + 1) * 128] for c in range(8)], masks)
            if dep is not None:
                qc = [c | dep for c in qc]
            q = [pltpu.bitcast(c, bf16).astype(f32) * Q_SCALE for c in qc]
            z = []
            for w in range(WIN):
                st = pl.ds(lb + HALO - DIL * w, R)
                zw = q[0] * kf_s[0, st, :]
                for j in range(1, 8):
                    zw = zw + q[j] * kf_s[j, st, :]
                zw = zw + jnp.where(odd, pltpu.roll(zw, 1, 1), pltpu.roll(zw, 127, 1))
                zw = zw + jnp.where(hi16, pltpu.roll(zw, 16, 1), pltpu.roll(zw, 112, 1))
                if w > 0:
                    zw = jnp.where(row >= DIL * w, zw, -1e9)
                z.append(zw)
            mx = z[0]
            for w in range(1, WIN):
                mx = jnp.maximum(mx, z[w])
            e = [jnp.exp2(zw - mx) for zw in z]
            den = e[0]
            for w in range(1, WIN):
                den = den + e[w]
            rden = 1.0 / den
            a = [ew * rden for ew in e]
            outs = []
            for j in range(8):
                o = a[0] * vf_s[j, pl.ds(lb + HALO, R), :]
                for w in range(1, WIN):
                    o = o + a[w] * vf_s[j, pl.ds(lb + HALO - DIL * w, R), :]
                outs.append(pltpu.bitcast(o.astype(bf16), i32))
            nat = _permute(outs, masks)
            for c in range(8):
                ob_d[pl.ds(b, R), c * 128:(c + 1) * 128] = pltpu.bitcast(nat[c], bf16)
            return pltpu.bitcast(a[0], i32)[0:R // 2, :]

        def trip(f, c):
            @pl.when(t == 0)
            def _():
                for cp in tcopies(f):
                    cp.wait()
            for k in range(SUB):
                ffn(xn_t, pl.multiple_of(FC0 + f * FT + k * FC, 128), FC, False)
            b0 = pl.multiple_of(f * RPT, RPT)
            zero = jnp.full((UNIT // 2, 128), jnp.minimum(f, 0), i32)
            dep = None
            for u in range(RPT // UNIT):
                bu = pl.multiple_of(b0 + u * UNIT, UNIT)
                if u == 0:
                    perm_kv(b0, 0, HALO + UNIT, None)
                else:
                    perm_kv(b0, HALO + u * UNIT, UNIT, dep)
                prev = dep
                dep = attn(bu, u * UNIT, dep) & zero
                rs = pl.ds(bu, UNIT)
                xi = xb_d[1 - slot, rs, :]
                if prev is not None:
                    xi = pltpu.bitcast(pltpu.bitcast(xi, i32) | jnp.concatenate([prev] * 8, axis=1), bf16)
                xn_d[1 - slot, rs, :] = _layernorm(xi)
            return c

        @pl.when(t + 1 < NT)
        def _():
            xcopy(t + 1).wait()
        jax.lax.fori_loop(0, NTRIP, trip, 0)

        @pl.when(t == 0)
        def _():
            wocopy().wait()

        @pl.when(t >= 2)
        def _():
            for r in range(len(OBS)):
                ocopy(t - 2, r).wait()

        raw_d[0:HALO, D:3 * D] = raw_d[TM:TM + HALO, D:3 * D]
        ss = [jnp.dot(ob_d[OST[r]:OST[r] + OBS[r], :], wo_d[...], preferred_element_type=f32)
              for r in range(len(OBS))]
        for r in range(len(OBS)):
            rs = slice(OST[r], OST[r] + OBS[r])
            out_d[slot, rs, :] = (xb_d[slot, rs, :].astype(f32) + ss[r] * _silu(acc_s[rs, :])).astype(bf16)
            ocopy(t, r).start()

        @pl.when(t + 2 < NT)
        def _():
            xcopy(t + 2).start()

        @pl.when(t + 1 < NT)
        def _():
            xn_n = xn_d.at[1 - slot]
            ffn(xn_n, 0, FC0, True)
            for part in range(3):
                cs = slice(part * D, (part + 1) * D)
                r = jnp.dot(xn_n[...], wqkv_d[:, cs], preferred_element_type=f32)
                raw_d[HALO:HALO + TM, cs] = r.astype(bf16)
        return carry

    jax.lax.fori_loop(0, NT, tile, 0)
    for t in range(NT - 2, NT):
        for r in range(len(OBS)):
            ocopy(t, r).wait()


@jax.jit
def pallas_recurrent_scan__sliding_local_dilated__glu_gated_swiglu__prompt_kernel(
    A_x: jax.Array,
    A_wqkv: jax.Array,
    A_wo: jax.Array,
    B_x: jax.Array,
    B_w1: jax.Array,
    B_w3: jax.Array,
    B_w2: jax.Array,
):
    del B_x
    anyspec = pl.BlockSpec(memory_space=pl.ANY)
    out = pl.pallas_call(
        _kernel,
        in_specs=[anyspec] * 6,
        out_specs=anyspec,
        out_shape=jax.ShapeDtypeStruct((S, D), bf16),
        scratch_shapes=[
            pltpu.VMEM((2, TM // 2, D), i32),
            pltpu.VMEM((D // 2, 3 * D), i32),
            pltpu.VMEM((D // 2, D), i32),
            pltpu.VMEM((D // 2, F), i32),
            pltpu.VMEM((D // 2, F), i32),
            pltpu.VMEM((F // 2, D), i32),
            pltpu.VMEM((2, TM // 2, D), i32),
            pltpu.VMEM((2, TM // 2, D), i32),
            pltpu.VMEM(((TM + HALO) // 2, 3 * D), i32),
            pltpu.VMEM((8, RPT + HALO, 128), f32),
            pltpu.VMEM((8, RPT + HALO, 128), f32),
            pltpu.VMEM((TM // 2, D), i32),
            pltpu.VMEM((TM, D), f32),
            pltpu.SemaphoreType.DMA((XP,)),
            pltpu.SemaphoreType.DMA((2,)),
            pltpu.SemaphoreType.DMA((2, len(OBS))),
            pltpu.SemaphoreType.DMA((3, NP)),
            pltpu.SemaphoreType.DMA((NQ,)),
            pltpu.SemaphoreType.DMA((3, NTRIP + 1)),
        ],
        compiler_params=pltpu.CompilerParams(
            vmem_limit_bytes=110 * 2**20,
            flags={"XLA_TPU_EVENLY_DISTRIBUTE_CRITICAL_NODES": True},
        ),
    )(A_x[0], A_wqkv, A_wo, B_w1, B_w3, B_w2)
    return out[None]
```

```python
import jax
import jax.numpy as jnp
import numpy as np
from jax.experimental import pallas as pl
from jax.experimental.pallas import tpu as pltpu

S, D, F = 2048, 1024, 3584
HEAD_DIM, WIN, DIL = 32, 8, 2
f32, bf16, i32 = jnp.float32, jnp.bfloat16, jnp.int32

TM = 512
NT = S // TM
HALO = 16
NTRIP = 4
FT = F // NTRIP
SUBS = (512, 384)
RPT = TM // NTRIP
UNIT = 16
QP = ((0, 256, 2), (512, 512, 1), (1024, 1024, 2))
NQ = sum(n for _, _, n in QP)
XP, LNR = 2, 128
XR = TM // XP
OBS = (256, 192, 64)
OST = (0, 256, 448)
Q_SCALE = float(HEAD_DIM ** -0.5 * np.log2(np.e))


def _field_masks(shape):
    lane = jax.lax.broadcasted_iota(i32, shape, len(shape) - 1)
    fld = (lane >> 1) & 7
    return [((fld >> b) & 1) == 1 for b in range(3)]


def _permute(cols, masks):
    r = [cols[c] if c == 0 else pltpu.roll(cols[c], 2 * c, 1) for c in range(8)]
    x = [r[(-c) % 8] for c in range(8)]
    for b in range(3):
        x = [jnp.where(masks[b], x[(j - (1 << b)) % 8], x[j]) for j in range(8)]
    return [x[j] if j == 0 else pltpu.roll(x[j], 128 - 2 * j, 1) for j in range(8)]


def _silu(g):
    hg = 0.5 * g
    return hg + hg * jnp.tanh(hg)


def _layernorm(x):
    x = x.astype(f32)
    m = jnp.mean(x, axis=-1, keepdims=True)
    xc = x - m
    var = jnp.mean(xc * xc, axis=-1, keepdims=True)
    return (xc * jax.lax.rsqrt(var + 1e-5)).astype(bf16)


def _kernel(x_hbm, wqkv_hbm, wo_hbm, w1_hbm, w3_hbm, w2_hbm, o_hbm,
            xb, wqkv_s, wo_s, w1_s, w3_s, w2_s, out_s, xn_s, raw_s, kf_s, vf_s, ob_s, acc_s,
            x0sem, xsem, osem, qsem, tsem):
    xb_d, wqkv_d, wo_d, w1_d, w3_d, w2_d, out_d, xn_d, raw_d, ob_d = [
        r.bitcast(bf16) for r in (xb, wqkv_s, wo_s, w1_s, w3_s, w2_s, out_s, xn_s, raw_s, ob_s)]

    def x0copy(p):
        rs = pl.ds(pl.multiple_of(p * XR, XR), XR)
        return pltpu.make_async_copy(x_hbm.at[rs, :], xb_d.at[0, rs, :], x0sem.at[p])

    def xcopy(t):
        return pltpu.make_async_copy(x_hbm.at[pl.ds(pl.multiple_of(t * TM, TM), TM), :],
                                     xb_d.at[t & 1], xsem.at[t & 1])

    def ocopy(t, r):
        return pltpu.make_async_copy(out_d.at[t & 1, pl.ds(OST[r], OBS[r]), :],
                                     o_hbm.at[pl.ds(pl.multiple_of(t * TM + OST[r], 16), OBS[r]), :],
                                     osem.at[t & 1, r])

    def tcopies(f):
        sl = pl.ds(pl.multiple_of(f * FT, 128), FT)
        return [pltpu.make_async_copy(w1_hbm.at[:, sl], w1_d.at[:, sl], tsem.at[0, f]),
                pltpu.make_async_copy(w3_hbm.at[:, sl], w3_d.at[:, sl], tsem.at[1, f]),
                pltpu.make_async_copy(w2_hbm.at[sl, :], w2_d.at[sl, :], tsem.at[2, f])]

    def qcols(g, i):
        start, width, _ = QP[g]
        return pl.ds(pl.multiple_of(start + i * width, 128), width)

    def qcopy(g, i):
        base = sum(n for _, _, n in QP[:g])
        return pltpu.make_async_copy(wqkv_hbm.at[:, qcols(g, i)], wqkv_d.at[:, qcols(g, i)], qsem.at[base + i])

    def wocopy():
        return pltpu.make_async_copy(wo_hbm, wo_d, tsem.at[0, NTRIP])

    def ffn(xn, start, n, fresh):
        sl = pl.ds(start, n)
        g = jnp.dot(xn[...], w1_d[:, sl], preferred_element_type=f32)
        u = jnp.dot(xn[...], w3_d[:, sl], preferred_element_type=f32)
        h = (_silu(g) * u).astype(bf16)
        d = jnp.dot(h, w2_d[sl, :], preferred_element_type=f32)
        if fresh is None:
            acc_s[...] += d
        else:
            acc_s[...] = jnp.where(fresh, 0.0, acc_s[...]) + d

    for p in range(XP):
        x0copy(p).start()
    for g in range(len(QP)):
        for i in range(QP[g][2]):
            qcopy(g, i).start()
    xcopy(1).start()
    for c in tcopies(0) + tcopies(1):
        c.start()
    raw_d[0:HALO, D:3 * D] = jnp.zeros((HALO, 2 * D), bf16)

    def zero_acc(i, c):
        acc_s[pl.ds(pl.multiple_of(i * 64, 64), 64), :] = jnp.zeros((64, D), f32)
        return c
    jax.lax.fori_loop(0, TM // 64, zero_acc, 0)

    def pro_ln(p, c):
        x0copy(p).wait()

        def rows(i, c2):
            rs = pl.ds(pl.multiple_of(p * XR + i * LNR, LNR), LNR)
            xn_d[0, rs, :] = _layernorm(xb_d[0, rs, :])
            return c2
        jax.lax.fori_loop(0, XR // LNR, rows, 0)
        return c
    jax.lax.fori_loop(0, XP, pro_ln, 0)

    for g in range(len(QP)):
        def pro_qkv(i, c, g=g):
            qcopy(g, i).wait()
            r = jnp.dot(xn_d[0], wqkv_d[:, qcols(g, i)], preferred_element_type=f32)
            raw_d[HALO:HALO + TM, qcols(g, i)] = r.astype(bf16)
            return c
        if QP[g][2] == 1:
            pro_qkv(0, 0)
        else:
            jax.lax.fori_loop(0, QP[g][2], pro_qkv, 0)
        if g == 0:
            for f in range(2, NTRIP):
                for c in tcopies(f):
                    c.start()
            wocopy().start()

    def tile(t, carry):
        slot = t & 1
        xn_t = xn_d.at[slot]

        def perm_kv(b, r0, n, dep):
            masks = _field_masks((n // 2, 128))
            for part, dst in ((1, kf_s), (2, vf_s)):
                ri = pltpu.bitcast(raw_d[pl.ds(pl.multiple_of(b + r0, 16), n), part * D:(part + 1) * D], i32)
                cols = [ri[:, c * 128:(c + 1) * 128] for c in range(8)]
                if dep is not None:
                    cols = [c | dep for c in cols]
                cols = _permute(cols, masks)
                for j in range(8):
                    dst[j, r0:r0 + n, :] = pltpu.bitcast(cols[j], bf16).astype(f32)

        def attn(b, lb, dep):
            R = UNIT
            row = jax.lax.broadcasted_iota(i32, (R, 128), 0) + (t * TM + b)
            lane = jax.lax.broadcasted_iota(i32, (R, 128), 1)
            odd = (lane & 1) == 1
            hi16 = (lane & 16) != 0
            masks = _field_masks((R // 2, 128))
            qi = pltpu.bitcast(raw_d[pl.ds(pl.multiple_of(b + HALO, 16), R), 0:D], i32)
            qc = _permute([qi[:, c * 128:(c + 1) * 128] for c in range(8)], masks)
            if dep is not None:
                qc = [c | dep for c in qc]
            q = [pltpu.bitcast(c, bf16).astype(f32) * Q_SCALE for c in qc]
            z = []
            for w in range(WIN):
                st = pl.ds(lb + HALO - DIL * w, R)
                zw = q[0] * kf_s[0, st, :]
                for j in range(1, 8):
                    zw = zw + q[j] * kf_s[j, st, :]
                zw = zw + jnp.where(odd, pltpu.roll(zw, 1, 1), pltpu.roll(zw, 127, 1))
                zw = zw + jnp.where(hi16, pltpu.roll(zw, 16, 1), pltpu.roll(zw, 112, 1))
                if w > 0:
                    zw = jnp.where(row >= DIL * w, zw, -1e9)
                z.append(zw)
            mx = z[0]
            for w in range(1, WIN):
                mx = jnp.maximum(mx, z[w])
            e = [jnp.exp2(zw - mx) for zw in z]
            den = e[0]
            for w in range(1, WIN):
                den = den + e[w]
            rden = 1.0 / den
            a = [ew * rden for ew in e]
            outs = []
            for j in range(8):
                o = a[0] * vf_s[j, pl.ds(lb + HALO, R), :]
                for w in range(1, WIN):
                    o = o + a[w] * vf_s[j, pl.ds(lb + HALO - DIL * w, R), :]
                outs.append(pltpu.bitcast(o.astype(bf16), i32))
            nat = _permute(outs, masks)
            for c in range(8):
                ob_d[pl.ds(b, R), c * 128:(c + 1) * 128] = pltpu.bitcast(nat[c], bf16)
            return pltpu.bitcast(a[0], i32)[0:R // 2, :]

        def trip(f, c):
            @pl.when(t == 0)
            def _():
                for cp in tcopies(f):
                    cp.wait()
            off = 0
            for k, width in enumerate(SUBS):
                ffn(xn_t, pl.multiple_of(f * FT + off, 128), width, (f == 0) if k == 0 else None)
                off += width
            b0 = pl.multiple_of(f * RPT, RPT)
            zero = jnp.full((UNIT // 2, 128), jnp.minimum(f, 0), i32)
            dep = None
            for u in range(RPT // UNIT):
                bu = pl.multiple_of(b0 + u * UNIT, UNIT)
                if u == 0:
                    perm_kv(b0, 0, HALO + UNIT, None)
                else:
                    perm_kv(b0, HALO + u * UNIT, UNIT, dep)
                prev = dep
                dep = attn(bu, u * UNIT, dep) & zero
                rs = pl.ds(bu, UNIT)
                xi = xb_d[1 - slot, rs, :]
                if prev is not None:
                    xi = pltpu.bitcast(pltpu.bitcast(xi, i32) | jnp.concatenate([prev] * 8, axis=1), bf16)
                xn_d[1 - slot, rs, :] = _layernorm(xi)
            return c

        @pl.when(t + 1 < NT)
        def _():
            xcopy(t + 1).wait()
        jax.lax.fori_loop(0, NTRIP, trip, 0)

        @pl.when(t == 0)
        def _():
            wocopy().wait()

        @pl.when(t >= 2)
        def _():
            for r in range(len(OBS)):
                ocopy(t - 2, r).wait()

        raw_d[0:HALO, D:3 * D] = raw_d[TM:TM + HALO, D:3 * D]
        ss = [jnp.dot(ob_d[OST[r]:OST[r] + OBS[r], :], wo_d[...], preferred_element_type=f32)
              for r in range(len(OBS))]
        for r in range(len(OBS)):
            rs = slice(OST[r], OST[r] + OBS[r])
            out_d[slot, rs, :] = (xb_d[slot, rs, :].astype(f32) + ss[r] * _silu(acc_s[rs, :])).astype(bf16)
            ocopy(t, r).start()

        @pl.when(t + 2 < NT)
        def _():
            xcopy(t + 2).start()

        @pl.when(t + 1 < NT)
        def _():
            xn_n = xn_d.at[1 - slot]
            for part in range(3):
                cs = slice(part * D, (part + 1) * D)
                r = jnp.dot(xn_n[...], wqkv_d[:, cs], preferred_element_type=f32)
                raw_d[HALO:HALO + TM, cs] = r.astype(bf16)
        return carry

    jax.lax.fori_loop(0, NT, tile, 0)
    for t in range(NT - 2, NT):
        for r in range(len(OBS)):
            ocopy(t, r).wait()


@jax.jit
def pallas_recurrent_scan__sliding_local_dilated__glu_gated_swiglu__prompt_kernel(
    A_x: jax.Array,
    A_wqkv: jax.Array,
    A_wo: jax.Array,
    B_x: jax.Array,
    B_w1: jax.Array,
    B_w3: jax.Array,
    B_w2: jax.Array,
):
    del B_x
    anyspec = pl.BlockSpec(memory_space=pl.ANY)
    out = pl.pallas_call(
        _kernel,
        in_specs=[anyspec] * 6,
        out_specs=anyspec,
        out_shape=jax.ShapeDtypeStruct((S, D), bf16),
        scratch_shapes=[
            pltpu.VMEM((2, TM // 2, D), i32),
            pltpu.VMEM((D // 2, 3 * D), i32),
            pltpu.VMEM((D // 2, D), i32),
            pltpu.VMEM((D // 2, F), i32),
            pltpu.VMEM((D // 2, F), i32),
            pltpu.VMEM((F // 2, D), i32),
            pltpu.VMEM((2, TM // 2, D), i32),
            pltpu.VMEM((2, TM // 2, D), i32),
            pltpu.VMEM(((TM + HALO) // 2, 3 * D), i32),
            pltpu.VMEM((8, RPT + HALO, 128), f32),
            pltpu.VMEM((8, RPT + HALO, 128), f32),
            pltpu.VMEM((TM // 2, D), i32),
            pltpu.VMEM((TM, D), f32),
            pltpu.SemaphoreType.DMA((XP,)),
            pltpu.SemaphoreType.DMA((2,)),
            pltpu.SemaphoreType.DMA((2, len(OBS))),
            pltpu.SemaphoreType.DMA((NQ,)),
            pltpu.SemaphoreType.DMA((3, NTRIP + 1)),
        ],
        compiler_params=pltpu.CompilerParams(
            vmem_limit_bytes=110 * 2**20,
            flags={"XLA_TPU_EVENLY_DISTRIBUTE_CRITICAL_NODES": True},
        ),
    )(A_x[0], A_wqkv, A_wo, B_w1, B_w3, B_w2)
    return out[None]
```
